```python
import os as _os
_os.environ.setdefault('JAX_PLATFORMS', 'cpu')
import jax
import jax.numpy as jnp

def _softmax(x, axis=-1):
    return jax.nn.softmax(x, axis=axis)

def _gelu(x):
    return jax.nn.gelu(x, approximate=True)

def _silu(x):
    return jax.nn.silu(x)

def _sigmoid(x):
    return jax.nn.sigmoid(x)

def _layernorm(x, axis=-1, eps=1e-05):
    m = jnp.mean(x, axis=axis, keepdims=True)
    v = jnp.var(x, axis=axis, keepdims=True)
    return (x - m) / jnp.sqrt(v + eps)

def _scatter_add(tgt, idx, src, axis=0):
    return tgt.at[idx].add(src)

def _segment_sum(src, seg, n):
    return jax.ops.segment_sum(src, seg, n)

class _Rng:

    def __init__(self, key):
        self._k = key

    def _next(self):
        self._k, sub = jax.random.split(self._k)
        return sub

    def normal(self, shape):
        return jax.random.normal(self._next(), shape, dtype=jnp.bfloat16)

    def randint(self, lo, hi, shape):
        return jax.random.randint(self._next(), shape, lo, hi, dtype=jnp.int32)

    def uniform(self, shape, lo=0.0, hi=1.0):
        return jax.random.uniform(self._next(), shape, jnp.bfloat16, lo, hi)

    def permutation(self, n):
        return jax.random.permutation(self._next(), n)
kernel_name = 'recurrent_scan__memory_aug_recurrent_mem_tr__mixer_gmlp__prompt'

def setup_inputs():
    _rng = _Rng(jax.random.key(int.from_bytes(__import__("os").urandom(4), "little")))
    _w = lambda a: (lambda t: t.astype(jnp.bfloat16) if jnp.issubdtype(t.dtype, jnp.floating) else t)(jnp.asarray(a))

    def _A_setup():
        B, S, Dm = (1, 2048, 640)
        H, Dh = (32, 128)
        M, seg = (8, 32)
        seg = min(seg, S)
        S = S // seg * seg
        return {'x': _w((lambda *s: _rng.normal(s) * 0.05)(B, S, Dm)), 'mem0': _w((lambda *s: _rng.normal(s) * 0.1)(B, M, Dm)), 'Wq': _w((lambda *s: _rng.normal(s) * 1.6)(Dm, H, Dh) * Dm ** (-0.5)), 'Wk': _w((lambda *s: _rng.normal(s) * 1.6)(Dm, H, Dh) * Dm ** (-0.5)), 'Wv': _w((lambda *s: _rng.normal(s) * 0.1)(Dm, H, Dh) * Dm ** (-0.5)), 'Wo': _w((lambda *s: _rng.normal(s) * 0.1)(H, Dh, Dm) * (H * Dh) ** (-0.5)), 'seg_len': seg}
    _A_in = _A_setup()

    def _B_setup():
        B, S, D, F = (1, 2048, 640, 1728)
        Fh = F // 2
        return {'x': _w((lambda *s: _rng.normal(s) * 0.05)(B, S, D)), 'w_in': _w((lambda *s: _rng.normal(s) * 0.8)(D, 2 * Fh)), 'w_sp': _w(0.01 * (lambda *s: _rng.normal(s) * 0.8)(S, S)), 'b_sp': _w(1.0 + 0.01 * (lambda *s: _rng.normal(s) * 0.05)(S)), 'w_out': _w((lambda *s: _rng.normal(s) * 0.05)(Fh, D))}
    _B_in = _B_setup()
    return {'A_x': _A_in['x'], 'A_mem0': _A_in['mem0'], 'A_Wq': _A_in['Wq'], 'A_Wk': _A_in['Wk'], 'A_Wv': _A_in['Wv'], 'A_Wo': _A_in['Wo'], 'A_seg_len': _A_in['seg_len'], 'B_x': _B_in['x'], 'B_w_in': _B_in['w_in'], 'B_w_sp': _B_in['w_sp'], 'B_b_sp': _B_in['b_sp'], 'B_w_out': _B_in['w_out']}

def reference(A_x, A_mem0, A_Wq, A_Wk, A_Wv, A_Wo, A_seg_len, B_x, B_w_in, B_w_sp, B_b_sp, B_w_out):

    def _A_ref(x, mem0, Wq, Wk, Wv, Wo, seg_len):
        B, S, Dm = x.shape
        H, Dh = (Wq.shape[1], Wq.shape[2])
        M = mem0.shape[1]
        scale = Dh ** (-0.5)
        n_seg = S // seg_len
        L = M + seg_len
        idx = jnp.arange(L)
        mask = (idx[:, None] < M) | (idx[:, None] >= idx[None, :])
        mem = mem0
        outs = []
        for s in range(n_seg):
            xs = x[:, s * seg_len:(s + 1) * seg_len, :].copy()
            h = jnp.concatenate([mem, xs], axis=1)
            q = jnp.einsum('btd,dhe->bhte', h, Wq)
            k = jnp.einsum('btd,dhe->bhte', h, Wk)
            v = jnp.einsum('btd,dhe->bhte', h, Wv)
            scores = jnp.einsum('bhqe,bhke->bhqk', q, k) * scale
            scores = jnp.where(mask[None, None], scores, -1000000000.0)
            p = _softmax(scores, axis=-1)
            o = jnp.einsum('bhqk,bhke->bhqe', p, v)
            o = jnp.einsum('bhte,hed->btd', o, Wo)
            mem = o[:, :M, :].copy()
            outs.append(o[:, M:, :])
        return jnp.concatenate(outs, axis=1)

    def _B_ref(x, w_in, w_sp, b_sp, w_out):
        B, S, D = x.shape
        F = w_in.shape[-1]
        Fh = F // 2
        z = _gelu(jnp.einsum('bsd,df->bsf', x, w_in))
        z1 = z[..., :Fh].copy()
        z2 = _layernorm(z[..., Fh:], axis=-1)
        g = jnp.einsum('ts,bsf->btf', w_sp, z2) + b_sp[None, :, None]
        return jnp.einsum('bsf,fd->bsd', z1 * g, w_out)
    x = A_x
    xn = _layernorm(x, axis=-1)
    s = _A_ref(xn, A_mem0, A_Wq, A_Wk, A_Wv, A_Wo, A_seg_len)
    g = _silu(_B_ref(xn, B_w_in, B_w_sp, B_b_sp, B_w_out))
    return x + s * g
```

```python
import functools
import jax
import jax.numpy as jnp
import numpy as np
from jax import lax
import jax.experimental.pallas as pl
import jax.experimental.pallas.tpu as pltpu

F32 = jnp.float32
BF16 = jnp.bfloat16
U32 = jnp.uint32
NT = (((1,), (1,)), ((), ()))
LANES = 128


def _dot(a, b):
    return jnp.dot(a, b, preferred_element_type=F32)


def _dot_nt(a, b):
    return lax.dot_general(a, b, NT, preferred_element_type=F32)


def _gelu(a):
    u = a * (0.7978845608028654 + (0.7978845608028654 * 0.044715) * (a * a))
    return (0.5 * a) * (1.0 + jnp.tanh(u))


def _layernorm(a, axis):
    c = a - jnp.mean(a, axis=axis, keepdims=True)
    v = jnp.mean(c * c, axis=axis, keepdims=True)
    return c * lax.rsqrt(v + 1e-5)


def _kernel(x_hbm, mem0_ref, wq_hbm, wk_hbm, wv_hbm, wo_hbm, win_hbm, wsp_hbm, bsp_ref, wout_hbm,
            out_hbm,
            x_v, xn_v, xb_v, win_v, wsp_v, wout_v, z1_v, z2_v, u_v,
            wraw_v, wqkv_v, wo_v, out_v,
            sem_x, sem_win, sem_wsp, sem_w, sem_wo, sem_wout, sem_out, *, seg, H, opts):
    S, D = x_v.shape
    M = mem0_ref.shape[1]
    Dh = wq_hbm.shape[1]
    F = win_v.shape[0]
    Fh = F // 2
    Fp = u_v.shape[1]
    L = M + seg
    n_seg = S // seg
    ND = D // LANES
    TB = opts.get("tb", 512)
    n1 = S // TB
    TT = opts.get("tt", 256)
    n2 = S // TT
    DC = D // n2
    HP = H // 2

    def cp_x(i):
        r = pl.ds(pl.multiple_of(i * TB, TB), TB)
        return pltpu.make_async_copy(x_hbm.at[0, r], x_v.at[r], sem_x.at[i])

    def cp_win(i):
        r = pl.ds(i * Fh, Fh)
        return pltpu.make_async_copy(win_hbm.at[r], win_v.at[r], sem_win.at[i])

    def cp_wsp(i):
        r = pl.ds(pl.multiple_of(i * TT, TT), TT)
        return pltpu.make_async_copy(wsp_hbm.at[r], wsp_v.at[r], sem_wsp.at[i])

    def cp_w(t, i):
        r = pl.ds(pl.multiple_of(i * DC * HP, DC * HP), DC * HP)
        src = (wq_hbm, wk_hbm, wv_hbm)[t].bitcast(U32)
        return pltpu.make_async_copy(src.at[r], wraw_v.at[t, r], sem_w.at[t * n2 + i])

    def cp_wo(j):
        return pltpu.make_async_copy(wo_hbm.bitcast(U32).at[:, pl.ds(j * LANES, LANES)], wo_v.at[j], sem_wo.at[j])

    def cp_wout(j):
        return pltpu.make_async_copy(wout_hbm.bitcast(U32).at[:, pl.ds(j * LANES, LANES)],
                                     wout_v.at[j, pl.ds(0, Fh // 2)], sem_wout.at[j])

    def cp_out(s):
        r = pl.ds(pl.multiple_of(s * seg, seg), seg)
        return pltpu.make_async_copy(out_v.at[r], out_hbm.at[0, r], sem_out)

    cp_x(0).start()
    cp_win(1).start()
    cp_win(0).start()
    cp_x(1).start()

    wout_v[:, pl.ds(Fh // 2, (Fp - Fh) // 2), :] = jnp.zeros((ND, (Fp - Fh) // 2, LANES), U32)

    def ln_x(i):
        r = pl.ds(pl.multiple_of(i * TB, TB), TB)
        xn = _layernorm(x_v[r, :].astype(F32), -1)
        xn_v[r, :] = xn
        xb_v[r, :] = xn.astype(BF16)

    cp_x(0).wait()
    ln_x(0)
    cp_win(1).wait()
    cp_win(0).wait()

    per = n2 // n1

    def b1(i, carry):
        @pl.when(i + 2 < n1)
        def _():
            cp_x(i + 2).start()
        for p in range(per):
            cp_wsp(i * per + p).start()
            for t in range(3):
                cp_w(t, i * per + p).start()
        nxt = jnp.minimum(i + 1, n1 - 1)

        @pl.when(i + 1 < n1)
        def _():
            cp_x(i + 1).wait()
        r = pl.ds(pl.multiple_of(i * TB, TB), TB)
        xb = xb_v[r, :]
        z2 = _gelu(_dot_nt(win_v[pl.ds(Fh, Fh), :], xb))
        z2_v[:, r] = _layernorm(z2, 0).astype(BF16)
        z1 = _gelu(_dot_nt(win_v[pl.ds(0, Fh), :], xb))
        z1_v[:, r] = z1.astype(z1_v.dtype)
        ln_x(nxt)
        return carry
    lax.fori_loop(0, n1, b1, 0)

    for j in range(ND):
        cp_wout(j).start()
    for j in range(ND):
        cp_wo(j).start()

    bias = bsp_ref

    def b2(i, carry):
        cp_wsp(i).wait()
        for t in range(3):
            cp_w(t, i).wait()
        r = pl.ds(pl.multiple_of(i * TT, TT), TT)
        g = _dot_nt(z2_v[...], wsp_v[r, :]) + bias[:, r].astype(F32)
        ut = z1_v[:, r].astype(F32) * g
        ut = jnp.concatenate([ut, jnp.zeros((Fp - Fh, TT), F32)], axis=0)
        u_v[r, :] = ut.T.astype(BF16)
        ro = pl.ds(pl.multiple_of(i * (DC // 2), DC // 2), DC // 2)
        for t in range(3):
            blk = wraw_v.at[t, pl.ds(pl.multiple_of(i * DC * HP, DC * HP), DC * HP)]
            for j in range(HP):
                w = blk[pl.ds(j, DC, stride=HP), :]
                lo = pltpu.bitcast(w << 16, F32).astype(BF16)
                hi = pltpu.bitcast(w & jnp.uint32(0xFFFF0000), F32).astype(BF16)
                wqkv_v[t, 2 * j, ro] = pltpu.bitcast(lo, U32)
                wqkv_v[t, 2 * j + 1, ro] = pltpu.bitcast(hi, U32)
        return carry
    lax.fori_loop(0, n2, b2, 0)

    for j in range(ND):
        cp_wout(j).wait()
    for j in range(ND):
        cp_wo(j).wait()

    scale = Dh ** (-0.5)
    G = opts.get("G", 4)
    NG = H // G
    U = opts.get("unroll", 1)
    lq, lp, lo_ = opts.get("lags", (1, 2, 3))
    ypos = opts.get("ypos", NG + lo_)

    def step(s, mem):
        r = pl.ds(pl.multiple_of(s * seg, seg), seg)
        row = lax.broadcasted_iota(jnp.int32, (L, L), 0)
        col = lax.broadcasted_iota(jnp.int32, (L, L), 1)
        mask = (row < M) | (row >= col)
        h = jnp.concatenate([mem, xn_v[r, :]], axis=0)
        qkv, sc, pr, oo = {}, {}, {}, {}
        acc = [None] * ND
        gate = [None] * ND

        def do_qkv(g):
            for hd in range(g * G, (g + 1) * G):
                qkv[hd] = tuple(_dot(h, pltpu.bitcast(wqkv_v[t, hd], BF16)) for t in range(3))

        def do_qk(g):
            for hd in range(g * G, (g + 1) * G):
                q, k, v = qkv[hd]
                sc[hd] = _dot_nt(q, k.astype(BF16))

        def do_sm(g):
            for hd in range(g * G, (g + 1) * G):
                z = jnp.where(mask, sc[hd] * scale, -1e9)
                e = jnp.exp(z - jnp.max(z, axis=-1, keepdims=True))
                pr[hd] = e * pl.reciprocal(jnp.sum(e, axis=-1, keepdims=True), approx=False)

        def do_pv(g):
            for hd in range(g * G, (g + 1) * G):
                oo[hd] = _dot(pr[hd], qkv[hd][2].astype(BF16))

        def do_o(g):
            for hd in range(g * G, (g + 1) * G):
                for j in range(ND):
                    d = _dot(oo[hd], pltpu.bitcast(wo_v[j, pl.ds(hd * (Dh // 2), Dh // 2)], BF16))
                    acc[j] = d if acc[j] is None else acc[j] + d

        def do_y():
            u = u_v[r, :]
            for j in range(ND):
                y = _dot(u, pltpu.bitcast(wout_v[j], BF16))
                gate[j] = y * jax.nn.sigmoid(y)

        for t in range(NG + lo_ + 1):
            if t == ypos: do_y()
            if t < NG: do_qkv(t)
            if 0 <= t - lq < NG: do_qk(t - lq)
            if 0 <= t - lp < NG: do_sm(t - lp); do_pv(t - lp)
            if 0 <= t - lo_ < NG: do_o(t - lo_)
        o = jnp.concatenate(acc, axis=1)
        gt = jnp.concatenate(gate, axis=1)
        out_v[r, :] = (x_v[r, :].astype(F32) + o[M:, :] * gt).astype(BF16)
        cp_out(s).start()
        return o[:M, :]

    def steps(i, mem):
        for k in range(U):
            mem = step(i * U + k, mem)
        return mem

    lax.fori_loop(0, n_seg // U, steps, mem0_ref[0].astype(F32))
    pltpu.make_async_copy(out_v, out_hbm.at[0], sem_out).wait()


def build(opts):
    @functools.partial(jax.jit, static_argnames=("A_seg_len",))
    def fn(A_x, A_mem0, A_Wq, A_Wk, A_Wv, A_Wo, A_seg_len, B_x, B_w_in, B_w_sp, B_b_sp, B_w_out):
        del B_x
        B, S, D = A_x.shape
        H, Dh = A_Wq.shape[1], A_Wq.shape[2]
        F = B_w_in.shape[1]
        Fh = F // 2
        Fp = -(-Fh // LANES) * LANES
        n1 = S // opts.get("tb", 512)
        n2 = S // opts.get("tt", 256)
        ND = D // LANES
        any_spec = pl.BlockSpec(memory_space=pl.ANY)
        vm = pl.BlockSpec(memory_space=pltpu.VMEM)
        dma = pltpu.SemaphoreType.DMA
        scratch = [
            pltpu.VMEM((S, D), BF16),
            pltpu.VMEM((S, D), F32),
            pltpu.VMEM((S, D), BF16),
            pltpu.VMEM((F, D), BF16),
            pltpu.VMEM((S, S), BF16),
            pltpu.VMEM((ND, Fp // 2, LANES), U32),
            pltpu.VMEM((Fh, S), opts.get("z1dt", BF16)),
            pltpu.VMEM((Fh, S), BF16),
            pltpu.VMEM((S, Fp), BF16),
            pltpu.VMEM((3, D * H // 2, Dh), U32),
            pltpu.VMEM((3, H, D // 2, Dh), U32),
            pltpu.VMEM((ND, H * Dh // 2, LANES), U32),
            pltpu.VMEM((S, D), BF16),
            dma((n1,)), dma((2,)), dma((n2,)), dma((3 * n2,)), dma((ND,)), dma((ND,)), dma(()),
        ]
        return pl.pallas_call(
            functools.partial(_kernel, seg=A_seg_len, H=H, opts=opts),
            out_shape=jax.ShapeDtypeStruct((B, S, D), A_x.dtype),
            in_specs=[any_spec, vm, any_spec, any_spec, any_spec, any_spec, any_spec, any_spec, vm, any_spec],
            out_specs=any_spec,
            scratch_shapes=scratch,
            compiler_params=pltpu.CompilerParams(vmem_limit_bytes=120 * 2**20, flags=opts.get("flags")),
        )(A_x, A_mem0, A_Wq.reshape(D * H, Dh), A_Wk.reshape(D * H, Dh), A_Wv.reshape(D * H, Dh),
          A_Wo.reshape(H * Dh, D), B_w_in.T, B_w_sp, B_b_sp.reshape(1, S), B_w_out)
    return fn


pallas_recurrent_scan__memory_aug_recurrent_mem_tr__mixer_gmlp__prompt_kernel = build({'lags':(1,2,5),'unroll':2})
```

```python
import functools
import jax
import jax.numpy as jnp
import numpy as np
from jax import lax
import jax.experimental.pallas as pl
import jax.experimental.pallas.tpu as pltpu

F32 = jnp.float32
BF16 = jnp.bfloat16
U32 = jnp.uint32
NT = (((1,), (1,)), ((), ()))
LANES = 128
SUB = 8
EPS = 1e-5
LOG2E = 1.4426950408889634


STRASSEN = (
    (((0, 0, 1), (0, 1, 1)), ((1, 1, 1),), ((0, 0, -1), (0, 1, 1))),
    (((0, 0, 1),), ((0, 1, 1), (1, 1, -1)), ((0, 1, 1), (1, 1, 1))),
    (((1, 0, 1), (1, 1, 1)), ((0, 0, 1),), ((1, 0, 1), (1, 1, -1))),
    (((1, 1, 1),), ((1, 0, 1), (0, 0, -1)), ((0, 0, 1), (1, 0, 1))),
    (((0, 0, 1), (1, 1, 1)), ((0, 0, 1), (1, 1, 1)), ((0, 0, 1), (1, 1, 1))),
    (((0, 1, 1), (1, 1, -1)), ((1, 0, 1), (1, 1, 1)), ((0, 0, 1),)),
    (((1, 0, 1), (0, 0, -1)), ((0, 0, 1), (0, 1, 1)), ((1, 1, 1),)),
)


def _block_sum(blocks, terms, f):
    h = len(blocks) // 2
    quad = lambda r, c: [row[c * h:(c + 1) * h] for row in blocks[r * h:(r + 1) * h]]
    first = quad(*terms[0][:2])
    if len(terms) == 1:
        return first
    return [[f(terms[1][2], x, y) for x, y in zip(rx, ry)] for rx, ry in zip(first, quad(*terms[1][:2]))]


def _signed(sign, x, y):
    return x + y if sign > 0 else x - y


def _lhs_sums(blocks):
    if len(blocks) == 1:
        return [blocks[0][0]]
    return [v for terms, _, _ in STRASSEN for v in _lhs_sums(_block_sum(blocks, terms, _signed))]


def _dot(a, b):
    return jnp.dot(a, b, preferred_element_type=F32)


def _dot_nt(a, b):
    return lax.dot_general(a, b, NT, preferred_element_type=F32)


def _gelu2(a):
    u = a * (0.7978845608028654 + (0.7978845608028654 * 0.044715) * (a * a))
    return a * (1.0 + jnp.tanh(u))


def _ds(start, size):
    if isinstance(start, int):
        return pl.ds(start, size)
    return pl.ds(pl.multiple_of(start, size), size)


def _kernel(x_hbm, mem0_hbm, wq_hbm, wk_hbm, wv_hbm, wo_hbm, win_hbm, wsp_hbm, bsp_hbm, wout_hbm,
            out_hbm,
            x_v, xn_v, win_v, wsp_v, wout_v, z1_v, z2_v, zm_v, zc_v, u_v,
            wraw_v, wqkv_v, wo_v, out_v, kv_v, row_s, mem0_v, bsp_v,
            sem_x0, sem_x, sem_win, sem_wsp, sem_w, sem_late, sem_out, *, seg, S, H, opts):
    D = x_v.shape[1]
    M = mem0_hbm.shape[1]
    Dh = wq_hbm.shape[3]
    F = win_hbm.shape[0]
    Fh = F // 2
    Fq = Fh // 2
    NP = u_v.shape[0]
    L = M + seg
    n_seg = S // seg
    ND = D // LANES
    TB = opts.get("tb", 512)
    n1 = S // TB
    NC = TB // LANES
    TT = 2 * LANES * opts.get("pairs", 2)
    n2 = S // TT
    DC = D // n2
    HP = H // 2
    NA = HP // SUB
    LV = opts.get("lv", 2)
    NB = 2 ** LV
    FB = Fh // NB

    def cp_x0(c):
        r = pl.ds(c * LANES, LANES)
        return pltpu.make_async_copy(x_hbm.at[0, r], x_v.at[r], sem_x0.at[c])

    def cp_x(i):
        return pltpu.make_async_copy(x_hbm.at[0, _ds(i % n1 * TB, TB)], x_v.at[_ds(i * TB, TB)], sem_x.at[i - 1])

    def cp_win(i, j):
        r = pl.ds(i * Fq, Fq)
        return pltpu.make_async_copy(win_hbm.bitcast(U32).at[r, pl.ds(j * LANES, LANES)], win_v.at[j, r], sem_win.at[i])

    NTT = S // LANES

    def cp_wsp(j):
        return pltpu.make_async_copy(wsp_hbm.bitcast(U32).at[:, _ds(j * LANES, LANES)], wsp_v.at[j], sem_wsp)

    def cp_w(ta, par, i):
        t, a = divmod(ta, NA)
        r = pl.ds(i * DC // 2, DC // 2)
        src = (wq_hbm, wk_hbm, wv_hbm)[t].bitcast(U32).at[r, par, pl.ds(a * SUB, SUB)]
        dst = wraw_v.reshape(6 * NA, wraw_v.shape[1] // SUB, SUB, Dh).at[2 * ta + par, r]
        return pltpu.make_async_copy(src, dst, sem_w.at[i])

    def cp_ws(i):
        return [cp_w(ta, par, i) for ta in range(3 * NA) for par in range(2)]

    Fw = Fq // LANES * LANES
    Fr = Fq - Fw
    f_parts = [(0, 0, Fw), (Fq, Fw, Fw), (Fw, 2 * Fw, Fr), (Fq + Fw, 2 * Fw + Fr, Fr)]
    cp_late = [pltpu.make_async_copy(wout_hbm.bitcast(U32).at[pl.ds(src // 2, n // 2), pl.ds(j * LANES, LANES)],
                                     wout_v.at[j, pl.ds(dst // 2, n // 2)], sem_late)
               for j in range(ND) for src, dst, n in f_parts]
    cp_late += [pltpu.make_async_copy(wo_hbm.bitcast(U32).at[:, pl.ds(j * LANES, LANES)], wo_v.at[j], sem_late)
                for j in range(ND)]
    cp_late.append(pltpu.make_async_copy(mem0_hbm, mem0_v, sem_late))
    cp_bias = pltpu.make_async_copy(bsp_hbm, bsp_v, sem_win.at[0])

    U = opts.get("unroll", 4)

    def cp_out(s):
        r = _ds(s * seg * U, seg * U)
        return pltpu.make_async_copy(out_v.at[r], out_hbm.at[0, r], sem_out)

    for c in range(NC):
        cp_x0(c).start()
    for j in range(ND):
        cp_win(1, j).start()

    wout_v[:, pl.ds(Fq, NP * LANES // 2 - Fq), :] = jnp.zeros((ND, NP * LANES // 2 - Fq, LANES), U32)
    KS = (kv_v.shape[0] - 4 * SUB) // (2 * H)
    for j in range(2 * H):
        kv_v[pl.ds(j * KS, SUB), :] = jnp.zeros((SUB, Dh), F32)

    def ln_x(start, rows):
        r = _ds(start, rows)
        x = x_v[r, :].astype(F32)
        c = x - jnp.mean(x, axis=-1, keepdims=True)
        v = jnp.mean(c * c, axis=-1, keepdims=True)
        xn_v[r, :] = c * lax.rsqrt(v + EPS)

    with jax.named_scope('start'):
        for c in range(NC):
            cp_x0(c).wait()
            ln_x(c * LANES, LANES)
    with jax.named_scope('waitwin'):
        for j in range(ND):
            cp_win(1, j).wait()
    cp_x(1).start()

    def hidden(half, i):
        if isinstance(i, list):
            for b in i:
                yield from hidden(half, b)
            return
        def w_cols(lo, hi):
            rows = pl.ds(half * Fq, Fq)
            return jnp.concatenate([pltpu.bitcast(win_v[j, rows], BF16) for j in range(lo, hi)], axis=1)
        kk = (ND - 1) * LANES
        last = _dot_nt(w_cols(ND - 1, ND), xn_v[_ds(i * TB, TB), pl.ds(kk, LANES)].astype(BF16))
        xb = [xn_v[_ds(i * TB + c * LANES, LANES), pl.ds(0, kk)].astype(BF16) for c in range(NC)]
        yield -1, last[:, :LANES]
        for c in range(NC):
            yield c, _dot_nt(w_cols(0, ND - 1), xb[c]) + last[:, c * LANES:(c + 1) * LANES]

    def p1(i, carry):
        RL = opts.get("rl", 32)
        MID = opts.get("mid", 1)
        NL = opts.get("nl", NC - 2)
        npc = TB // NL // RL
        for c, pre in hidden(1, i):
            if c < 0:
                continue
            z = _gelu2(pre)
            z2_v[i * NC + c, pl.ds(0, Fh), :] = z
            zm_v[i * NC + c] = jnp.broadcast_to(jnp.mean(z, axis=0, keepdims=True), (SUB, LANES))
            if c == MID:
                cp_x(i + 1).wait()
                cp_x(jnp.minimum(i + 2, n1 + 1)).start()
            if MID <= c < MID + NL:
                for m in range(npc):
                    r0 = (m * Fh // npc) // 16 * 16
                    x_v[_ds(S + 2 * TB + (i % 2) * 16, 16), pl.ds(0, LANES)] = pre[r0:r0 + 16].astype(BF16)
                    ln_x((i + 1) * TB + ((c - MID) * npc + m) * RL, RL)

        @pl.when(i == 0)
        def _():
            for j in range(ND):
                cp_win(0, j).start()
            cp_bias.start()

        @pl.when(i > 0)
        def _():
            for j in range(NTT // n1):
                cp_wsp((i - 1) * (NTT // n1) + j).start()
        return carry
    if not opts.get('aonly'):
      with jax.named_scope('P1'):
        lax.fori_loop(0, n1, p1, 0)

    for j in range(ND):
        cp_win(0, j).wait()
    cp_bias.wait()
    for j in range(NTT // n1 * (n1 - 1), NTT):
        cp_wsp(j).start()

    U2 = opts.get("u2", 1)

    def p2(ii, carry):
      for i in [ii * U2 + b for b in range(U2)]:
        for p in range(n2 // n1):
            for cp in cp_ws(i * (n2 // n1) + p):
                cp.start()
        var, rstd = {}, {}
        rows = range(0, FB, SUB)
        work = []
        for g in range(NC // NB):
            work += [("var", g, r) for r in rows] + [("rstd", g, 0)] + [("norm", g, r) for r in rows]
        nvar = opts.get("nvar", 14)
        for c, pre in hidden(0, i):
            if c >= 0:
                z1_v[i * NC + c] = _gelu2(pre)
            mine = work[:nvar] if c < 0 else work[nvar:][c * (len(work) - nvar) // NC:(c + 1) * (len(work) - nvar) // NC]
            for m, (kind, g, r) in enumerate(mine):
                t0 = i * NC + g * NB
                if kind == "rstd":
                    for e in range(NB):
                        ss = jnp.broadcast_to(jnp.sum(var[g, e], axis=0, keepdims=True), (SUB, LANES))
                        rstd[g, e] = 0.5 * lax.rsqrt(ss * (1.0 / Fh) + 4.0 * EPS)
                    continue
                r0 = m * Fh // len(mine) // SUB * SUB
                z2_v[i % 3, pl.ds(Fh, SUB), :] = pre[r0:r0 + SUB]
                a = [[z2_v[t0 + e, pl.ds(f * FB + r, SUB), :] - zm_v[t0 + e] for e in range(NB)] for f in range(NB)]
                if kind == "var":
                    for e in range(NB):
                        sq = functools.reduce(lambda x, y: x + y, [a[f][e] * a[f][e] for f in range(NB)])
                        var[g, e] = var[g, e] + sq if (g, e) in var else sq
                else:
                    a = [[a[f][e] * rstd[g, e] for e in range(NB)] for f in range(NB)]
                    burst = opts.get("burst", 7)
                    for q, val in enumerate(_lhs_sums(a)):
                        if q and q % burst == 0:
                            r1 = (m * Fh + Fh * q // 7 ** LV) // len(mine) // SUB * SUB
                            zc_v[7 ** LV, i % 3, pl.ds(0, SUB), :] = pre[r1:r1 + SUB]
                        zc_v[q, i * (NC // NB) + g, pl.ds(r, SUB), :] = val
      return carry
    if not opts.get('aonly'):
      with jax.named_scope('P2'):
        lax.fori_loop(0, n1 // U2, p2, 0)

    for c in cp_late:
        c.start()
    for j in range(NTT):
        cp_wsp(j).wait()

    RC = opts.get("rc", 16)

    def p3(i, carry):
        for cp in cp_ws(i):
            cp.wait()

        def relayout(t, j, e):
            a, jj = divmod(j, SUB)
            rows = _ds((i * DC + e * RC) // 2 * SUB, RC // 2 * SUB)
            even, odd = [wraw_v.at[2 * (t * NA + a) + par, rows][pl.ds(jj, RC // 2, stride=SUB), :] for par in range(2)]
            ro = _ds((i * DC + e * RC) // 2, RC // 2)
            wqkv_v[t, 2 * j, ro] = pltpu.pack_elementwise([even, odd], packed_dtype=jnp.uint16)
            wqkv_v[t, 2 * j + 1, ro] = (even >> 16) | (odd & jnp.uint32(0xFFFF0000))

        rl = [(t, j, e) for t in range(3) for j in range(HP) for e in range(DC // RC)]
        n_grp = TT // (NB * LANES)
        KJ = S // LANES // NB
        n_job = n_grp * 7 ** LV * (KJ // 4)
        state = [0]
        posts = []

        def leaf(q, rhs, emit):
            acc = None
            for h in range(KJ // 4):
                js = range(4 * h, 4 * h + 4)
                d = _dot_nt(jnp.concatenate([zc_v[q, j] for j in js], axis=1),
                            jnp.concatenate([packed(rhs[j]()) for j in js], axis=1))
                acc = d if acc is None else acc + d
                n = state[0]
                state[0] += 1
                mine = rl[n * len(rl) // n_job:(n + 1) * len(rl) // n_job]
                early = len(posts)
                if h == KJ // 4 - 1:
                    emit(0, 0, acc)
                for m, piece in enumerate(mine):
                    r0 = (m * FB // len(mine)) // SUB * SUB
                    tick = d[r0:r0 + SUB]
                    wraw_v[i % (3 * NA), pl.ds(D // 2 * SUB, SUB), :] = pltpu.bitcast(tick, U32)
                    relayout(*piece)
                    if early and m % opts.get("pp", 6) == 0:
                        u_v[i % NP, pl.ds(S, SUB), :] = tick
                        posts.pop(0)()
                        early -= 1

        def halves(w):
            if isinstance(w, tuple):
                return w
            return pltpu.bitcast(w << 16, F32), pltpu.bitcast(w & jnp.uint32(0xFFFF0000), F32)

        def packed(w):
            if isinstance(w, tuple):
                w = pltpu.pack_elementwise(list(w), packed_dtype=BF16)
            return pltpu.bitcast(w, BF16)

        def lazy_sum(sign, x, y):
            def one(a, b):
                memo = []

                def get():
                    if not memo:
                        memo.append(tuple(_signed(sign, p, q) for p, q in zip(halves(a()), halves(b()))))
                    return memo[0]
                return get
            return [one(a, b) for a, b in zip(x, y)]

        def products(q, rhs, emit):
            if len(rhs) == 1:
                return leaf(q, rhs[0][0], emit)
            h = len(rhs) // 2
            acc, left = {}, {}
            for _, _, outs in STRASSEN:
                for r, c, _ in outs:
                    left[r, c] = left.get((r, c), 0) + 1
            for p, (_, terms, outs) in enumerate(STRASSEN):
                for r, c, _ in outs:
                    left[r, c] -= 1

                def inner(r0, c0, val, outs=outs):
                    for r, c, sign in outs:
                        key = (r * h + r0, c * h + c0)
                        if key not in acc:
                            acc[key] = (sign, val)
                        elif acc[key][0] > 0:
                            acc[key] = (1, _signed(sign, acc[key][1], val))
                        else:
                            acc[key] = (sign, val - acc[key][1]) if sign > 0 else (-1, acc[key][1] + val)
                        if not left[r, c]:
                            emit(*key, acc.pop(key)[1])
                products(q * 7 + p, _block_sum(rhs, terms, lazy_sum), inner)

        for gi in range(n_grp):
            t0 = i * TT + gi * NB * LANES
            bias = 0.5 * bsp_v[_ds(t0, NB * LANES)].astype(F32).reshape(1, NB * LANES)
            g, todo = {}, []

            def w(e, c, j, t0=t0):
                return lambda: wsp_v[NB * j + e, _ds((t0 + c * LANES) // 2, LANES // 2), :]

            for c in range(NB):
                for f in range(2):
                    for j in range(Fw // LANES):
                        todo.append((f * (Fw // LANES) + j, c, [(f * Fq + j * LANES, f * Fq + (j + 1) * LANES)]))
                todo.append((NP - 1, c, [(Fw, Fq), (Fq + Fw, Fh)]))

            def post(p, c, spans, t0=t0, bias=bias, g=g):
                parts = []
                for lo, hi in spans:
                    for f in range(lo // FB, (hi - 1) // FB + 1):
                        a, b = max(lo, f * FB), min(hi, (f + 1) * FB)
                        z1 = z1_v[t0 // LANES + c, pl.ds(a, b - a), :]
                        parts.append(z1 * (g[f, c][a - f * FB:b - f * FB] + bias[:, c * LANES:(c + 1) * LANES]))
                n = sum(x.shape[0] for x in parts)
                if n < LANES:
                    parts.append(jnp.zeros((LANES - n, LANES), F32))
                u_v[p, _ds(t0 + c * LANES, LANES), :] = jnp.concatenate(parts, axis=0).T

            def finished(f, c, val, g=g, todo=todo, post=post):
                g[f, c] = val
                for item in list(todo):
                    need = {(ff, item[1]) for lo, hi in item[2] for ff in range(lo // FB, (hi - 1) // FB + 1)}
                    if need <= set(g):
                        todo.remove(item)
                        posts.append(functools.partial(post, *item))

            products(0, [[[w(e, c, j) for j in range(KJ)] for c in range(NB)] for e in range(NB)], finished)
        for p in posts:
            p()
        return carry
    if not opts.get('aonly'):
      with jax.named_scope('P3'):
        lax.fori_loop(0, n2, p3, 0)

    for c in cp_late:
        c.wait()
    cp_x(n1 + 1).wait()

    c2 = Dh ** (-0.5) * LOG2E
    NEG = -1e9 * LOG2E
    G = opts.get("G", 4)
    NG = H // G
    nvs = opts.get("nv", 1)
    if isinstance(nvs, int): nvs = [nvs] * NG
    nvs = [nvs[hd * len(nvs) // H] for hd in range(H)]

    row_s[0] = 2 * H * KS

    def tree(f, xs):
        w = opts.get("tw", 1)
        parts = [functools.reduce(f, xs[i::w]) for i in range(w)]
        return functools.reduce(f, parts)

    def recip(x):
        if opts.get("exact_rcp"):
            return pl.reciprocal(x, approx=False)
        r = pl.reciprocal(x, approx=True)
        return r * (2.0 - x * r)


    def schedule(last):
        ne, lag = opts.get("early", (3, 5))
        order = opts.get("inner", "xqpo")
        seq = []
        for t in range(NG):
            for w in order:
                if w == "x": seq.append(("qkv", t))
                if w == "q" and t >= 1: seq.append(("qk", t - 1))
                if w == "p" and t >= 2: seq.append(("pv", t - 2))
                if w == "o" and 0 <= t - lag < ne: seq.append(("o", t - lag))
        tail = opts.get("tail", "o3 q7 p6 o4 o5 p7 o6 y0 o7 y1 y2 y3 y4")
        if last:
            tail = opts.get("tail_last", "o3 q7 p6 o4 o5 p7 y0 y1 y2 y3 y4 o6 o7")
        names = dict(o="o", q="qk", p="pv", y="y")
        return seq + [(names[w[0]], int(w[1:])) for w in tail.split()]

    def step(s, mem, k):
        r = _ds(s * seg, seg)
        mask = {}
        for nv in sorted(set(nvs)):
            row = lax.broadcasted_iota(jnp.int32, (L - nv * SUB, L), 0)
            col = lax.broadcasted_iota(jnp.int32, (L - nv * SUB, L), 1)
            mask[nv] = (row < M) | (row + nv * SUB >= col)
        sub = lax.broadcasted_iota(jnp.int32, (SUB, 1), 0)
        h = jnp.concatenate([mem, xn_v[r, :]], axis=0)
        qkv, sc, pr, oo, vo = {}, {}, {}, {}, {}
        acc = [None] * ND
        gate = [None] * ND

        def vpu_unit(hd, a):
            q = qkv[hd][0]
            kbase = hd * 2 * KS + SUB
            vbase = kbase + KS
            r0 = M + a * SUB
            qs = q[r0:r0 + SUB] * c2
            ts = range(r0, -SUB, -1)
            z = [jnp.sum(qs * kv_v[pl.ds(kbase + t, SUB), :], axis=-1, keepdims=True) for t in ts]
            z = [zt if t >= 0 else jnp.where(sub >= -t, zt, NEG) for zt, t in zip(z, ts)]
            CK = opts.get("ck", 0) or len(z)
            mx = den = num = None
            for c0 in range(0, len(z), CK):
                zc, tc = z[c0:c0 + CK], ts[c0:c0 + CK]
                mc = tree(jnp.maximum, zc)
                new_mx = mc if mx is None else jnp.maximum(mx, mc)
                e = [jnp.exp2(zt - new_mx) for zt in zc]
                d = tree(lambda x, y: x + y, e)
                n = tree(lambda x, y: x + y, [et * kv_v[pl.ds(vbase + t, SUB), :] for et, t in zip(e, tc)])
                if mx is None:
                    den, num = d, n
                else:
                    alpha = jnp.exp2(mx - new_mx)
                    den, num = den * alpha + d, num * alpha + n
                mx = new_mx
            vo[hd, a] = num * recip(den)

        ready = []
        clock = [0.0]
        issued = [0.0]
        total = sum(M + (a + 1) * SUB for hd in range(H) for a in range(nvs[hd]))
        t_lo, t_hi = opts.get("pace", (66, 640))

        def tick(res, tiles, flush=None):
            clock[0] += tiles
            while ready and (ready[0][0] == flush or clock[0] >= t_lo + (t_hi - t_lo) * issued[0] / total):
                hd, a = ready.pop(0)
                if opts.get("tick", False):
                    kv_v[_ds(tick_row, SUB), :] = res[:SUB]
                vpu_unit(hd, a)
                issued[0] += M + (a + 1) * SUB

        def do_qkv(g):
            for hd in range(g * G, (g + 1) * G):
                res = []
                res = [None] * 3
                for t in opts.get("qkvo", (0, 1, 2)):
                    res[t] = _dot(h, pltpu.bitcast(wqkv_v[t, hd], BF16))
                    tick(res[t], ND)
                qkv[hd] = res
                nk = M + nvs[hd] * SUB
                if nvs[hd]:
                    kv_v[pl.ds(hd * 2 * KS + SUB, nk), :] = res[1][:nk]
                    kv_v[pl.ds(hd * 2 * KS + KS + SUB, nk), :] = res[2][:nk]
                    ready.extend((hd, a) for a in range(nvs[hd]))
                last[0] = res[0]

        def do_qk(g):
            for hd in range(g * G, (g + 1) * G):
                q, k, v = qkv[hd]
                qm = jnp.concatenate([q[:M], q[M + nvs[hd] * SUB:]], axis=0) if nvs[hd] else q
                sc[hd] = _dot_nt(qm, k.astype(BF16))
            clock[0] += G

        def do_pv(g):
            for hd in range(g * G, (g + 1) * G):
                z = jnp.where(mask[nvs[hd]], sc[hd] * c2, NEG)
                e = jnp.exp2(z - jnp.max(z, axis=-1, keepdims=True))
                p = e * recip(jnp.sum(e, axis=-1, keepdims=True))
                oo[hd] = _dot(p, qkv[hd][2].astype(BF16))
                tick(oo[hd], 1)

        def do_o(g):
            for hd in range(g * G, (g + 1) * G):
                tick(last[0], 0, flush=hd)
                o = oo[hd]
                if nvs[hd]:
                    o = jnp.concatenate([o[:M]] + [vo[hd, a] for a in range(nvs[hd])] + [o[M:]], axis=0)
                for j in range(ND):
                    d = _dot(o, pltpu.bitcast(wo_v[j, pl.ds(hd * (Dh // 2), Dh // 2)], BF16))
                    acc[j] = d if acc[j] is None else acc[j] + d
                    last[0] = d
                    tick(d, 1)

        def do_y(j):
            if not us:
                us.append(jnp.concatenate([u_v[p, r, :] for p in range(NP)], axis=1).astype(BF16))
            y = _dot(us[0], pltpu.bitcast(wout_v[j], BF16))
            hy = 0.5 * y
            gate[j] = hy + hy * jnp.tanh(hy)

        us = []
        last = [None]
        for op, g in schedule(k == U - 1):
            if op == "qkv": do_qkv(g)
            elif op == "qk": do_qk(g)
            elif op == "pv": do_pv(g)
            elif op == "o": do_o(g)
            elif op == "y": do_y(g)
        o = jnp.concatenate(acc, axis=1)
        gt = jnp.concatenate(gate, axis=1)
        out_v[r, :] = (x_v[r, :].astype(F32) + o[M:, :] * gt).astype(BF16)
        return o[:M, :]

    def steps(i, mem):
        for k in range(U):
            mem = step(i * U + k, mem, k)
        cp_out(i).start()
        return mem

    with jax.named_scope('A'):
        lax.fori_loop(0, n_seg // U, steps, mem0_v[0].astype(F32))
    with jax.named_scope('waitout'):
        pltpu.make_async_copy(out_v, out_hbm.at[0], sem_out).wait()


def build(opts):
    @functools.partial(jax.jit, static_argnames=("A_seg_len",))
    def fn(A_x, A_mem0, A_Wq, A_Wk, A_Wv, A_Wo, A_seg_len, B_x, B_w_in, B_w_sp, B_b_sp, B_w_out):
        del B_x
        B, S, D = A_x.shape
        H, Dh = A_Wq.shape[1], A_Wq.shape[2]
        F = B_w_in.shape[1]
        Fh = F // 2
        NP = -(-Fh // LANES)
        TB = opts.get("tb", 512)
        n1 = S // TB
        n2 = S // (2 * LANES * opts.get("pairs", 2))
        ND = D // LANES
        NTT = S // LANES
        LV = opts.get("lv", 2)
        any_spec = pl.BlockSpec(memory_space=pl.ANY)
        vm = pl.BlockSpec(memory_space=pltpu.VMEM)
        dma = pltpu.SemaphoreType.DMA
        scratch = [
            pltpu.VMEM((S + 2 * TB + 64, D), BF16),
            pltpu.VMEM((S + TB, D), F32),
            pltpu.VMEM((ND, F // 2, LANES), U32),
            pltpu.VMEM((NTT, S // 2, LANES), U32),
            pltpu.VMEM((ND, NP * LANES // 2, LANES), U32),
            pltpu.VMEM((NTT, Fh, LANES), F32),
            pltpu.VMEM((NTT, Fh + SUB, LANES), F32),
            pltpu.VMEM((NTT, SUB, LANES), F32),
            pltpu.VMEM((7 ** LV + 1, NTT // 2 ** LV, Fh // 2 ** LV, LANES), F32),
            pltpu.VMEM((NP, S + opts.get('pu', 32), LANES), F32),
            pltpu.VMEM((6 * H // 16, (D // 2 + 4) * SUB, Dh), U32),
            pltpu.VMEM((3, H, D // 2, Dh), U32),
            pltpu.VMEM((ND, H * Dh // 2, LANES), U32),
            pltpu.VMEM((S, D), BF16),
            pltpu.VMEM((H * 2 * 32 + 4 * SUB, Dh), F32),
            pltpu.SMEM((1,), jnp.int32),
            pltpu.VMEM(A_mem0.shape, BF16),
            pltpu.VMEM(B_b_sp.shape, BF16),
            dma((TB // LANES,)), dma((n1 + 1,)), dma((2,)), dma(()), dma((n2,)), dma(()), dma(()),
        ]
        return pl.pallas_call(
            functools.partial(_kernel, seg=A_seg_len, S=S, H=H, opts=opts),
            out_shape=jax.ShapeDtypeStruct((B, S, D), A_x.dtype),
            in_specs=[any_spec] * 10,
            out_specs=any_spec,
            scratch_shapes=scratch,
            compiler_params=pltpu.CompilerParams(vmem_limit_bytes=opts.get("vmem", 120) * 2**20, flags=opts.get("flags", {"XLA_TPU_RESCHEDULE_DMA_DONES": True}),
                                                 disable_bounds_checks=opts.get("nobc", True),
                                                 disable_semaphore_checks=opts.get("nosc", False)),
        )(A_x, A_mem0, *[w.reshape(D // 2, 2, H, Dh) for w in (A_Wq, A_Wk, A_Wv)], A_Wo.reshape(H * Dh, D), B_w_in.T, B_w_sp, B_b_sp, B_w_out)
    return fn


pallas_recurrent_scan__memory_aug_recurrent_mem_tr__mixer_gmlp__prompt_kernel = build({})
```

```python
import functools
import jax
import jax.numpy as jnp
import numpy as np
from jax import lax
import jax.experimental.pallas as pl
import jax.experimental.pallas.tpu as pltpu

F32 = jnp.float32
BF16 = jnp.bfloat16
U32 = jnp.uint32
NT = (((1,), (1,)), ((), ()))
LANES = 128
SUB = 8
EPS = 1e-5
LOG2E = 1.4426950408889634


STRASSEN = (
    (((0, 0, 1), (0, 1, 1)), ((1, 1, 1),), ((0, 0, -1), (0, 1, 1))),
    (((0, 0, 1),), ((0, 1, 1), (1, 1, -1)), ((0, 1, 1), (1, 1, 1))),
    (((1, 0, 1), (1, 1, 1)), ((0, 0, 1),), ((1, 0, 1), (1, 1, -1))),
    (((1, 1, 1),), ((1, 0, 1), (0, 0, -1)), ((0, 0, 1), (1, 0, 1))),
    (((0, 0, 1), (1, 1, 1)), ((0, 0, 1), (1, 1, 1)), ((0, 0, 1), (1, 1, 1))),
    (((0, 1, 1), (1, 1, -1)), ((1, 0, 1), (1, 1, 1)), ((0, 0, 1),)),
    (((1, 0, 1), (0, 0, -1)), ((0, 0, 1), (0, 1, 1)), ((1, 1, 1),)),
)


SUMS = tuple(p for p, (_, terms, _) in enumerate(STRASSEN) if len(terms) > 1)


def _block_sum(blocks, terms, f):
    h = len(blocks) // 2
    quad = lambda r, c: [row[c * h:(c + 1) * h] for row in blocks[r * h:(r + 1) * h]]
    first = quad(*terms[0][:2])
    if len(terms) == 1:
        return first
    return [[f(terms[1][2], x, y) for x, y in zip(rx, ry)] for rx, ry in zip(first, quad(*terms[1][:2]))]


def _signed(sign, x, y):
    return x + y if sign > 0 else x - y


def _halves(w):
    if isinstance(w, tuple):
        return w
    return pltpu.bitcast(w << 16, F32), pltpu.bitcast(w & jnp.uint32(0xFFFF0000), F32)


def _words(w):
    return pltpu.pack_elementwise(list(w), packed_dtype=BF16) if isinstance(w, tuple) else w


def _signed_halves(sign, x, y):
    return tuple(_signed(sign, p, q) for p, q in zip(_halves(x), _halves(y)))


def _strassen(h, product, emit, deferred=False):
    acc = {}
    for p, (_, _, outs) in enumerate(STRASSEN):
        later = {(r, c) for _, _, o in STRASSEN[p + 1:] for r, c, _ in o}

        def add(r0, c0, val, outs=outs, later=later):
            for r, c, sign in outs:
                key = (r * h + r0, c * h + c0)
                if key not in acc:
                    acc[key] = (sign, val)
                elif acc[key][0] > 0:
                    acc[key] = (1, _signed(sign, acc[key][1], val))
                else:
                    acc[key] = (1, val - acc[key][1]) if sign > 0 else (-1, acc[key][1] + val)
                if (r, c) not in later:
                    emit(*key, acc.pop(key)[1])
        product(p, add)


def _lhs_sums(blocks):
    if len(blocks) == 1:
        return [blocks[0][0]]
    return [v for terms, _, _ in STRASSEN for v in _lhs_sums(_block_sum(blocks, terms, _signed))]


def _dot(a, b):
    return jnp.dot(a, b, preferred_element_type=F32)


def _dot_nt(a, b):
    return lax.dot_general(a, b, NT, preferred_element_type=F32)


def _gelu2(a):
    u = a * (0.7978845608028654 + (0.7978845608028654 * 0.044715) * (a * a))
    return a * (1.0 + jnp.tanh(u))


def _ds(start, size):
    if isinstance(start, int):
        return pl.ds(start, size)
    return pl.ds(pl.multiple_of(start, size), size)


def _kernel(x_hbm, mem0_hbm, wq_hbm, wk_hbm, wv_hbm, wo_hbm, win_hbm, wsp_hbm, bsp_hbm, wout_hbm,
            out_hbm,
            x_v, xn_v, win_v, wsp_v, wout_v, z1_v, z2_v, zm_v, zc_v, u_v,
            wraw_v, wqkv_v, wo_v, out_v, kv_v, row_s, wsum_v, wqs_v, wys_v, mem0_v, bsp_v, pad_v,
            sem_x0, sem_x, sem_win, sem_wsp, sem_w, sem_late, sem_out, *, seg, S, H, opts):
    D = x_v.shape[1]
    M = mem0_hbm.shape[1]
    Dh = wq_hbm.shape[-1]
    F = win_hbm.shape[0]
    Fh = F // 2
    Fq = Fh // 2
    NP = u_v.shape[0]
    L = M + seg
    n_seg = S // seg
    ND = D // LANES
    TB = opts.get("tb", 512)
    n1 = S // TB
    NC = TB // LANES
    TT = 2 * LANES * opts.get("pairs", 2)
    n2 = S // TT
    DC = D // n2
    HP = H // 2
    NA = HP // SUB
    LV = opts.get("lv", 2)
    NB = 2 ** LV
    FB = Fh // NB

    XC = opts.get("xc", 256)

    def cp_x0(c):
        r = _ds(c * XC, XC)
        return pltpu.make_async_copy(x_hbm.at[0, r], x_v.at[r], sem_x0.at[c])

    def start_x(i):
        for c in range(0, TB, LANES):
            pltpu.make_async_copy(x_hbm.at[0, _ds(i * TB + c, LANES)], x_v.at[_ds(i * TB + c, LANES)],
                                  sem_x.at[i - 1]).start()

    def wait_x(i):
        blk = x_v.at[_ds(i * TB, TB)]
        pltpu.make_async_copy(blk, blk, sem_x.at[i - 1]).wait()

    def cp_win(i):
        r = pl.ds(i * Fh, Fh)
        return pltpu.make_async_copy(win_hbm.at[r], win_v.at[r], sem_win.at[i])

    NTT = S // LANES

    def cp_wsp(j):
        return pltpu.make_async_copy(wsp_hbm.bitcast(U32).at[:, _ds(j * LANES, LANES)], wsp_v.at[j], sem_wsp)

    KP = (ND - 1) // 2
    YP = (NP - 1) // 2
    OB = H * Dh // 2 // n2
    DT = LANES // n2

    def cp_ws(i):
        r = pl.ds(i * DT // 2, DT // 2)
        dst = wraw_v.reshape(wraw_v.shape[0], ND, LANES // 2, SUB, Dh)
        return [pltpu.make_async_copy(w.bitcast(U32).at[:, r, par, pl.ds(a * SUB, SUB)],
                                      dst.at[2 * (t * NA + a) + par, :, r], sem_w.at[i])
                for t, w in enumerate((wq_hbm, wk_hbm, wv_hbm)) for a in range(NA) for par in range(2)]

    Fw = Fq // LANES * LANES
    Fr = Fq - Fw
    f_parts = [(0, 0, Fw), (Fq, Fw, Fw), (Fw, 2 * Fw, Fr), (Fq + Fw, 2 * Fw + Fr, Fr)]
    cp_wout = [pltpu.make_async_copy(wout_hbm.bitcast(U32).at[pl.ds(src // 2, n // 2), pl.ds(j * LANES, LANES)],
                                     wout_v.at[j, pl.ds(dst // 2, n // 2)], sem_wsp)
               for j in range(ND) for src, dst, n in f_parts]
    cp_late = [pltpu.make_async_copy(wo_hbm.bitcast(U32).at[:, pl.ds(j * LANES, LANES)], wo_v.at[j], sem_late)
                for j in range(ND)]
    cp_late.append(pltpu.make_async_copy(mem0_hbm, mem0_v, sem_late))
    cp_bias = pltpu.make_async_copy(bsp_hbm, bsp_v, sem_win.at[0])

    U = opts.get("unroll", 4)

    def cp_out(s):
        r = _ds(s * seg * U, seg * U)
        return pltpu.make_async_copy(out_v.at[r], out_hbm.at[0, r], sem_out)

    def first_copies(f, carry):
        for c in range(TB // XC // 2):
            cp_x0(f * (TB // XC // 2) + c).start()
        r = _ds(Fh + f * Fq, Fq)
        pltpu.make_async_copy(win_hbm.at[r], win_v.at[r], sem_win.at[1]).start()
        return carry
    lax.fori_loop(0, 2, first_copies, 0)

    wout_v[:, pl.ds(Fq, NP * LANES // 2 - Fq), :] = jnp.zeros((ND, NP * LANES // 2 - Fq, LANES), U32)
    KS, NKV = opts.get("ks", 48), opts.get("nkv", 2)
    for j in range(2 * H * NKV):
        kv_v[pl.ds(j * KS, SUB), :] = jnp.zeros((SUB, Dh), F32)

    def ln_x(start, rows):
        r = _ds(start, rows)
        x = x_v[r, :].astype(F32)
        c = x - jnp.mean(x, axis=-1, keepdims=True)
        v = jnp.mean(c * c, axis=-1, keepdims=True)
        xn_v[r, :] = c * lax.rsqrt(v + EPS)

    def win_sums(half):
        tile = lambda f, r, j: pltpu.bitcast(
            win_v[pl.ds((2 * half + f) * Fq + 2 * r, 2 * SUB), pl.ds(j * LANES, LANES)], U32)
        for r in range(0, Fq // 2, SUB):
            for j in range(KP):
                raw = [[tile(f, r, k * KP + j) for k in range(2)] for f in range(2)]
                split = [[_halves(w) for w in row] for row in raw]
                for p, (terms, _, _) in enumerate(STRASSEN):
                    val = _block_sum(split if len(terms) > 1 else raw, terms, _signed_halves)[0][0]
                    wsum_v[half, p, j, pl.ds(r, SUB)] = _words(val)
            for f in range(2):
                wsum_v[half, 7, f, pl.ds(r, SUB)] = tile(f, r, ND - 1)

    def hidden(half, i, emit, busy):
        xn = lambda c, lo, n: xn_v[_ds(i * TB + c * LANES, LANES), pl.ds(lo * LANES, n * LANES)]
        w_last = pltpu.bitcast(jnp.concatenate([wsum_v[half, 7, f] for f in range(2)], axis=0), BF16)
        blocks = [[jnp.concatenate([xn(c, k * KP, KP) for c in range(c1, NC, 2)], axis=0) for c1 in range(2)]
                  for k in range(2)]
        last = _dot_nt(w_last, jnp.concatenate([xn(c, ND - 1, 1) for c in range(NC)], axis=0).astype(BF16))
        busy(0, last)

        def product(p, add):
            lhs = [wsum_v[half, p, j] for j in range(KP)]
            d = _dot_nt(jnp.concatenate([pltpu.bitcast(w, BF16) for w in lhs], axis=1),
                        _block_sum(blocks, STRASSEN[p][1], _signed)[0][0].astype(BF16))
            add(0, 0, d)
            busy(p + 1, d)

        def done(f, c1, val):
            for n, c in enumerate(range(c1, NC, 2)):
                emit(f, c, val[:, n * LANES:(n + 1) * LANES] + last[f * Fq:(f + 1) * Fq, c * LANES:(c + 1) * LANES])
        _strassen(1, product, done)

    def first_block(c, carry):
        cp_x0(c).wait()
        if opts.get("x1pos", 1) >= 0:
            @pl.when(c == opts.get("x1pos", 1))
            def _():
                start_x(1)
        ln_x(c * XC, XC)
        return carry
    with jax.named_scope('start'):
        lax.fori_loop(0, TB // XC, first_block, 0)
    with jax.named_scope('waitwin'):
        cp_win(1).wait()
    if opts.get("x1pos", 1) < 0:
        start_x(1)
    win_sums(1)

    def p1(i, carry):
        RL = opts.get("rl", 8)
        MID, END = opts.get("mid", (2, 7))
        sums = {}

        def emit(f, c, pre):
            z = _gelu2(pre)
            z2_v[i * NC + c, pl.ds(f * Fq, Fq), :] = z
            part = jnp.sum(z.reshape(Fq // SUB, SUB, LANES), axis=0)
            if c in sums:
                mean = jnp.sum(sums[c] + part, axis=0, keepdims=True) * (1.0 / Fh)
                zm_v[i * NC + c] = jnp.broadcast_to(mean, (SUB, LANES))
            sums[c] = part

        def busy(n, d):
            if n == MID:
                pl.when(i + 1 < n1)(lambda: wait_x(i + 1))
                first = opts.get("wsp0", 4)
                for it in range(n1):
                    @pl.when(i == it)
                    def _(it=it):
                        if it == 0:
                            for b in range(2, n1):
                                start_x(b)
                            cp_win(0).start()
                            cp_bias.start()
                        cut = lambda k: first + k * (NTT - first) // (n1 - 1) if k >= 0 else 0
                        for j in range(cut(it - 1), cut(it)):
                            cp_wsp(j).start()
            if MID <= n < END:
                mine = range((n - MID) * (TB // RL) // (END - MID), (n + 1 - MID) * (TB // RL) // (END - MID))
                for m, piece in enumerate(mine):
                    r0 = (m * d.shape[0] // len(mine)) // 16 * 16
                    x_v[_ds(S + (i % 2) * 16, 16), pl.ds(0, LANES)] = d[r0:r0 + 16, :LANES].astype(BF16)
                    ln_x(jnp.minimum(i + 1, n1 - 1) * TB + piece * RL, RL)
        hidden(1, i, emit, busy)

        return carry
    if not opts.get('aonly'):
      with jax.named_scope('P1'):
        lax.fori_loop(0, n1, p1, 0)

    cp_win(0).wait()
    cp_bias.wait()
    win_sums(0)
    for cp in cp_wout + cp_ws(0):
        cp.start()

    U2 = opts.get("u2", 1)

    def p2(ii, carry):
      for i in [ii * U2 + b for b in range(U2)]:
        var, rstd = {}, {}
        rows = range(0, FB, SUB)
        work = []
        for g in range(NC // NB):
            work += [("var", g, r) for r in rows] + [("rstd", g, 0)] + [("norm", g, r) for r in rows]
        nvar = opts.get("nvar", 28)

        def emit(f, c, pre):
            z1_v[i * NC + c, pl.ds(f * Fq, Fq), :] = _gelu2(pre)

        def busy(n, d):
            share = opts.get("share", (1, 2, 3, 4, 5, 6, 7))
            rest = len(work) - nvar
            cut = lambda k: nvar + (share[k - 1] * rest // share[-1] if k else 0)
            mine = work[cut(n - 1):cut(n)] if n else work[:nvar]
            for m, (kind, g, r) in enumerate(mine):
                t0 = i * NC + g * NB
                if kind == "rstd":
                    for e in range(NB):
                        ss = jnp.broadcast_to(jnp.sum(var[g, e], axis=0, keepdims=True), (SUB, LANES))
                        rstd[g, e] = 0.5 * lax.rsqrt(ss * (1.0 / Fh) + 4.0 * EPS)
                    continue
                r0 = m * d.shape[0] // len(mine) // SUB * SUB
                z2_v[i % 3, pl.ds(Fh, SUB), :] = d[r0:r0 + SUB, :LANES]
                a = [[z2_v[t0 + e, pl.ds(f * FB + r, SUB), :] - zm_v[t0 + e] for e in range(NB)] for f in range(NB)]
                if kind == "var":
                    for e in range(NB):
                        sq = functools.reduce(lambda x, y: x + y, [a[f][e] * a[f][e] for f in range(NB)])
                        var[g, e] = var[g, e] + sq if (g, e) in var else sq
                else:
                    a = [[a[f][e] * rstd[g, e] for e in range(NB)] for f in range(NB)]
                    burst = opts.get("burst", 11)
                    for q, val in enumerate(_lhs_sums(a)):
                        if q and q % burst == 0:
                            r1 = (m * 7 ** LV + q) * d.shape[0] // 7 ** LV // len(mine) // SUB * SUB
                            zc_v[7 ** LV, i % 3, pl.ds(0, SUB), :] = d[r1:r1 + SUB, :LANES]
                        zc_v[q, i * (NC // NB) + g, pl.ds(r, SUB), :] = val
        hidden(0, i, emit, busy)

        @pl.when(i == opts.get("w1", n1 - 1))
        def _():
            for cp in cp_ws(1) + cp_late[:1]:
                cp.start()

      return carry
    if not opts.get('aonly'):
      with jax.named_scope('P2'):
        lax.fori_loop(0, n1 // U2, p2, 0)

    for cp in [cp_wsp(j) for j in range(NTT)] + cp_wout:
        cp.wait()

    RC = opts.get("rc", 16)

    def p3(i, carry):
        with jax.named_scope('wW'):
            for cp in cp_ws(i):
                cp.wait()

        def raw(t, j, d):
            a, jj = divmod(j, SUB)
            rows = _ds(d // 2 * SUB, SUB * SUB)
            return [wraw_v.at[2 * (t * NA + a) + par, rows][pl.ds(jj, SUB, stride=SUB), :] for par in range(2)]

        def relayout(t, j, e):
            if t == -2:
                pair = i * (HP // n2) + j
                for n in range(KP):
                    blocks = [[_halves(wo_v[2 * n + c, _ds((2 * pair + k) * (Dh // 2) + e * SUB, SUB)]) for c in range(2)]
                              for k in range(2)]
                    for m, p in enumerate(SUMS):
                        val = _words(_block_sum(blocks, STRASSEN[p][1], _signed_halves)[0][0])
                        z2_v[pair, pl.ds((n * len(SUMS) + m) * (Dh // 2) + e * SUB, SUB), :] = pltpu.bitcast(val, F32)
            elif t < 0:
                r = i * (YP * LANES // 2 // n2) + e * SUB
                blocks = [[_halves(wout_v[c * KP + j, _ds(k * YP * LANES // 2 + r, SUB)]) for c in range(2)] for k in range(2)]
                for n, p in enumerate(SUMS):
                    wys_v[n, j, _ds(r, SUB)] = _words(_block_sum(blocks, STRASSEN[p][1], _signed_halves)[0][0])
            elif e >= 0:
                d = e // 2 * LANES + i * DT + e % 2 * 2 * SUB
                blocks = []
                for k in range(2):
                    even, odd = [_halves(w) for w in raw(t, j, k * KP * LANES + d)]
                    blocks.append([(even[c], odd[c]) for c in range(2)])
                    for c in range(2):
                        wqkv_v[t, 2 * j + c, _ds((k * KP * LANES + d) // 2, SUB)] = _words(blocks[k][c])
                for n, p in enumerate(SUMS):
                    wqs_v[t, j, n, _ds(d // 2, SUB)] = _words(_block_sum(blocks, STRASSEN[p][1], _signed_halves)[0][0])
            else:
                d = 2 * KP * LANES + i * DT + (-e - 1) * 2 * SUB
                even, odd = raw(t, j, d)
                wqkv_v[t, 2 * j, _ds(d // 2, SUB)] = pltpu.pack_elementwise([even, odd], packed_dtype=jnp.uint16)
                wqkv_v[t, 2 * j + 1, _ds(d // 2, SUB)] = (even >> 16) | (odd & jnp.uint32(0xFFFF0000))

        rl = [(t, j, e) for t in range(3) for j in range(HP)
              for e in opts.get("rlo", (0, 1, 2, 3, -1, -2))]
        extra = [(-1, j, e) for j in range(KP) for e in range(YP * LANES // 2 // n2 // SUB)]
        if opts.get("so", False):
            extra += [(-2, j, e) for j in range(HP // n2) for e in range(Dh // 2 // SUB)]
        for n, piece in enumerate(extra):
            rl.insert((n + 1) * len(rl) // (len(extra) + 1), piece)
        n_grp = TT // (NB * LANES)
        KJ = S // LANES // NB
        n_job = n_grp * 7 ** LV * (KJ // 4)
        state = [0]
        posts = []

        def leaf(q, rhs, emit):
            acc = None
            for h in range(KJ // 4):
                js = range(4 * h, 4 * h + 4)
                d = _dot_nt(jnp.concatenate([zc_v[q, j] for j in js], axis=1),
                            jnp.concatenate([pltpu.bitcast(_words(rhs[j]()), BF16) for j in js], axis=1))
                acc = d if acc is None else acc + d
                n = state[0]
                state[0] += 1
                mine = rl[n * len(rl) // n_job:(n + 1) * len(rl) // n_job]
                early = len(posts)
                if h == KJ // 4 - 1:
                    emit(0, 0, acc)
                for m, piece in enumerate(mine):
                    r0 = (m * FB // len(mine)) // SUB * SUB
                    tick = d[r0:r0 + SUB]
                    wraw_v[6 * NA, _ds(i * SUB, SUB), :] = pltpu.bitcast(tick, U32)
                    relayout(*piece)
                    if early and m % opts.get("pp", 3) == 0:
                        u_v[i % NP, pl.ds(S, SUB), :] = tick
                        posts.pop(0)()
                        early -= 1

        def lazy_sum(sign, x, y):
            def one(a, b):
                memo = []

                def get():
                    if not memo:
                        memo.append(_signed_halves(sign, a(), b()))
                    return memo[0]
                return get
            return [one(a, b) for a, b in zip(x, y)]

        def products(q, rhs, emit):
            if len(rhs) == 1:
                return leaf(q, rhs[0][0], emit)
            _strassen(len(rhs) // 2,
                      lambda p, add: products(q * 7 + p, _block_sum(rhs, STRASSEN[p][1], lazy_sum), add), emit)

        for gi in range(n_grp):
            t0 = i * TT + gi * NB * LANES
            bias = 0.5 * bsp_v[_ds(t0, NB * LANES)].astype(F32).reshape(1, NB * LANES)
            g, todo = {}, []

            def w(e, c, j, t0=t0):
                return lambda: wsp_v[NB * j + e, _ds((t0 + c * LANES) // 2, LANES // 2), :]

            for c in range(NB):
                for f in range(2):
                    for j in range(Fw // LANES):
                        todo.append((f * (Fw // LANES) + j, c, [(f * Fq + j * LANES, f * Fq + (j + 1) * LANES)]))
                todo.append((NP - 1, c, [(Fw, Fq), (Fq + Fw, Fh)]))

            def post(p, c, spans, t0=t0, bias=bias, g=g):
                parts = []
                for lo, hi in spans:
                    for f in range(lo // FB, (hi - 1) // FB + 1):
                        a, b = max(lo, f * FB), min(hi, (f + 1) * FB)
                        z1 = z1_v[t0 // LANES + c, pl.ds(a, b - a), :]
                        parts.append(z1 * (g[f, c][a - f * FB:b - f * FB] + bias[:, c * LANES:(c + 1) * LANES]))
                n = sum(x.shape[0] for x in parts)
                if n < LANES:
                    parts.append(jnp.zeros((LANES - n, LANES), F32))
                u_v[p, _ds(t0 + c * LANES, LANES), :] = jnp.concatenate(parts, axis=0).T

            def finished(f, c, val, g=g, todo=todo, post=post):
                g[f, c] = val
                for item in list(todo):
                    need = {(ff, item[1]) for lo, hi in item[2] for ff in range(lo // FB, (hi - 1) // FB + 1)}
                    if need <= set(g):
                        todo.remove(item)
                        posts.append(functools.partial(post, *item))

            products(0, [[[w(e, c, j) for j in range(KJ)] for c in range(NB)] for e in range(NB)], finished)
        for p in posts:
            p()

        for it, cps in enumerate((cp_ws(2) + cp_late[1:2], cp_ws(3) + cp_late[2:3], cp_late[3:])):
            @pl.when(i == it)
            def _(cps=cps):
                for cp in cps:
                    cp.start()

        return carry
    if not opts.get('aonly') and not opts.get('bonly'):
      with jax.named_scope('P3'):
        lax.fori_loop(0, n2, p3, 0)

    for c in cp_late:
        c.wait()

    c2 = Dh ** (-0.5) * LOG2E
    NEG = -1e9 * LOG2E
    G = opts.get("G", 4)
    NG = H // G
    GS = seg // SUB
    row_s[0] = 2 * H * KS

    def recip(x):
        r = pl.reciprocal(x, approx=True)
        return r * (2.0 - x * r)

    def chain(f, xs):
        return functools.reduce(f, xs)

    plain = [(False, range(k * GS, (k + 1) * GS)) for k in range(U)]
    q_plan = [(True, range(0, 7)), (False, range(7, 10)), (False, range(10, 13)), (False, range(13, 16))]
    o_plan = [(False, range(0, 3)), (False, range(3, 6)), (False, range(6, 9)), (True, range(9, 16))]
    if not opts.get("sq", True): q_plan = plain
    if opts.get("p64"): q_plan = [(False, g) for _, g in q_plan]
    if not opts.get("so", False): o_plan = plain
    if opts.get("lagged"):
        if opts.get("so", False):
            o_plan = [(False, (1, 2, 3)), (False, (0, 5, 6)), (False, (4, 7, 9)), (True, (8, 10, 11, 12, 13, 14, 15))]
        else:
            o_plan = [(False, (1, 2, 3)), (False, (0, 5, 6, 7)), (False, (4, 9, 10, 11)), (False, (8, 12, 13, 14, 15))]

    ahead = [g for k, (_, gs) in enumerate(q_plan) for g in gs if g >= (k + 1) * GS]

    def schedule(k):
        ne, lag = opts.get("early", (3, 5)) if k < U - 1 else opts.get("early_last", (3, 5))
        order = opts.get("inner", "xqpo")
        seq = []
        for t in range(NG):
            for w in order:
                if w == "x": seq.append(("qkv", t))
                if w == "q" and t >= 1: seq.append(("qk", t - 1))
                if w == "p" and t >= 2: seq.append(("pv", t - 2))
                if w == "o" and 0 <= t - lag < ne: seq.append(("o", t - lag))
        tail = opts.get("tail", "o3 q7 p6 o4 o5 p7 o6 y0 o7 y1 y2 y3 y4")
        if k == U - 1:
            tail = opts.get("tail_last", "o3 q7 p6 y0 y1 o4 p7 o5 y2 y3 y4 o6 o7")
        names = dict(o="o", q="qk", p="pv", y="y")
        return seq + [(names[w[0]], int(w[1:])) for w in tail.split()]

    def groups(a):
        return [a[r:r + SUB] for r in range(0, a.shape[0], SUB)]

    def rows(parts):
        return jnp.concatenate(parts, axis=0)

    def lhs(a, kind):
        return a.astype(BF16) if a.shape[0] % (2 * SUB) == 0 and kind in opts.get("pack", "h") else a

    def period(i, mem):
        row = lax.broadcasted_iota(jnp.int32, (L - SUB, L), 0)
        col = lax.broadcasted_iota(jnp.int32, (L - SUB, L), 1)
        mask = (row < M) | (row + SUB >= col)
        sub = lax.broadcasted_iota(jnp.int32, (SUB, 1), 0)
        proj = {}
        att = {}
        gate, res, gating = {}, {}, []

        tokens = _ds(i * U * seg, U * seg)
        xn_p, x_p, u_p, out_p = xn_v.at[tokens], x_v.at[tokens], u_v.at[:, tokens], out_v.at[tokens]

        def xn(g):
            return xn_p[pl.ds(g * SUB, SUB), :]

        for k in range(U):
            fast_q, qg = q_plan[k]
            fast_o, og = o_plan[k]
            qg, og = ["m"] + list(qg), ["m"] + list(og)
            keys = ["m"] + list(range(k * GS, (k + 1) * GS))
            h = rows([mem] + [xn(g) for g in qg[1:]])
            sc, acc, us = {}, {}, []
            if fast_q:
                n = h.shape[0] // 2
                blocks = [[h[f * n:(f + 1) * n, c * KP * LANES:(c + 1) * KP * LANES] for c in range(2)] for f in range(2)]
                h_sums = [lhs(_block_sum(blocks, terms, _signed)[0][0], 'h') for terms, _, _ in STRASSEN]
            h = lhs(h, 'h')

            def keep(t, hd, names, vals):
                for g, val in zip(names, vals):
                    if g in keys or not opts.get("carry", True):
                        proj[t, hd, g] = val
                    else:
                        z1_v[8 + ahead.index(g), pl.ds((t * H + hd) * SUB, SUB), :] = val
                for g in keys:
                    if g not in names and opts.get("carry", True):
                        proj[t, hd, g] = z1_v[8 + ahead.index(g), pl.ds((t * H + hd) * SUB, SUB), :]

            def weight(ref, *idx):
                return pltpu.bitcast(ref[idx], BF16)

            def project(t, j):
                if not fast_q:
                    for hd in (2 * j, 2 * j + 1):
                        keep(t, hd, qg, groups(_dot(h, weight(wqkv_v, t, hd))))
                    return
                tail = pl.ds(KP * LANES, LANES // 2)
                last = [_dot(h[:, (ND - 1) * LANES:], weight(wqkv_v, t, 2 * j + c, tail)) for c in range(2)]

                def product(p, add):
                    terms = STRASSEN[p][1]
                    if len(terms) > 1:
                        w = weight(wqs_v, t, j, SUMS.index(p))
                    else:
                        w = weight(wqkv_v, t, 2 * j + terms[0][1], pl.ds(terms[0][0] * KP * LANES // 2, KP * LANES // 2))
                    add(0, 0, _dot(h_sums[p], w))

                def done(f, c, val):
                    n = val.shape[0]
                    parts[c, f] = groups(val + last[c][f * n:(f + 1) * n])
                parts = {}
                _strassen(1, product, done)
                for c in range(2):
                    keep(t, 2 * j + c, qg, parts[c, 0] + parts[c, 1])

            def first_rows(hd):
                kbase = (k % NKV * H + hd) * 2 * KS + SUB
                vbase = kbase + KS
                nk = len(keys) if opts.get("allkv", 1) else 2
                kv_v[pl.ds(kbase, nk * SUB), :] = rows([proj[1, hd, g] for g in keys[:nk]])
                kv_v[pl.ds(vbase, nk * SUB), :] = rows([proj[2, hd, g] for g in keys[:nk]])
                if opts.get("stq", 1):
                    slab, n0 = divmod(k % 2 * H + hd, Fh // L)
                    z1_v[slab, pl.ds(n0 * L, L), :] = rows([proj[0, hd, g] for g in keys])
                    for n, g in enumerate(keys):
                        proj[0, hd, g] = z1_v[slab, pl.ds(n0 * L + n * SUB, SUB), :]
                if opts.get("allkv", 1):
                    for n, g in enumerate(keys):
                        proj[1, hd, g] = kv_v[pl.ds(kbase + n * SUB, SUB), :]
                        proj[2, hd, g] = kv_v[pl.ds(vbase + n * SUB, SUB), :]
                qs = proj[0, hd, keys[1]] * c2
                ts = range(M, -SUB, -1)
                z = [jnp.sum(qs * kv_v[pl.ds(kbase + t, SUB), :], axis=-1, keepdims=True) for t in ts]
                z = [zt if t >= 0 else jnp.where(sub >= -t, zt, NEG) for zt, t in zip(z, ts)]
                mx = chain(jnp.maximum, z)
                e = [jnp.exp2(zt - mx) for zt in z]
                den = chain(jnp.add, e)
                num = chain(jnp.add, [et * kv_v[pl.ds(vbase + t, SUB), :] for et, t in zip(e, ts)])
                att[hd, keys[1]] = num * recip(den)

            def do_qkv(g):
                for j in range(g * G // 2, (g + 1) * G // 2):
                    for t in opts.get("qkvo", (0, 1, 2)):
                        project(t, j)
                    for hd in (2 * j, 2 * j + 1):
                        first_rows(hd)

            def do_qk(g):
                for hd in range(g * G, (g + 1) * G):
                    q = rows([proj[0, hd, r] for r in keys[:1] + keys[2:]])
                    sc[hd] = _dot_nt(lhs(q, 'q'), rows([proj[1, hd, r] for r in keys]).astype(BF16))

            def do_pv(g):
                for hd in range(g * G, (g + 1) * G):
                    z = jnp.where(mask, sc[hd] * c2, NEG)
                    e = jnp.exp2(z - jnp.max(z, axis=-1, keepdims=True))
                    p = e * recip(jnp.sum(e, axis=-1, keepdims=True))
                    o = _dot(lhs(p, 'p'), rows([proj[2, hd, r] for r in keys]).astype(BF16))
                    att.update(zip([(hd, r) for r in keys[:1] + keys[2:]], groups(o)))

            def accumulate(key, d):
                if opts.get("accv"):
                    slot = key if isinstance(key, int) else ND + key[0] * KP + key[1]
                    r = pl.ds(slot * 64 if slot < ND else ND * 64 + (slot - ND) * 32, d.shape[0])
                    z1_v[14 + k % 2, r, :] = z1_v[14 + k % 2, r, :] + d if key in acc else d
                    acc[key] = functools.partial(lambda r: z1_v[14 + k % 2, r, :], r)
                else:
                    acc[key] = acc[key] + d if key in acc else d

            def do_o(g):
                for j in range(g * G // 2, (g + 1) * G // 2):
                    o = [rows([att[2 * j + c, r] for r in og]) for c in range(2)]
                    head = lambda c: pl.ds((2 * j + c) * (Dh // 2), Dh // 2)
                    if not fast_o:
                        for c in range(2):
                            a = lhs(o[c], 'o')
                            for n in range(ND):
                                accumulate(n, _dot(a, weight(wo_v, n, head(c))))
                        continue
                    half = o[0].shape[0] // 2
                    blocks = [[o[c][f * half:(f + 1) * half] for c in range(2)] for f in range(2)]
                    for c in range(2):
                        accumulate(ND - 1, _dot(lhs(o[c], 'o'), weight(wo_v, ND - 1, head(c))))
                    for p, (left, terms, _) in enumerate(STRASSEN):
                        a = lhs(_block_sum(blocks, left, _signed)[0][0], 'o')
                        for n in range(KP):
                            if len(terms) > 1:
                                w = pltpu.bitcast(z2_v[j, pl.ds((n * len(SUMS) + SUMS.index(p)) * (Dh // 2), Dh // 2), :], BF16)
                            else:
                                w = weight(wo_v, 2 * n + terms[0][1], head(terms[0][0]))
                            accumulate((p, n), _dot(a, w))

            def silu(n, names, y):
                hy = 0.5 * y
                gate.update(zip([(n, r) for r in names], groups(hy + hy * jnp.tanh(hy))))

            def do_y(j):
                if not opts.get("sy", True):
                    if not us:
                        us.append(jnp.concatenate([u_p[p, pl.ds(k * seg, seg), :] for p in range(NP)], axis=1).astype(BF16))
                    silu(j, keys[1:], _dot(us[0], weight(wout_v, j)))
                    return
                if k % 2 == 0 and j == 0:
                    gating[:] = gate_jobs(k)
                if gating:
                    gating.pop(0)()

            def gate_jobs(k):
                both = pl.ds(k * seg, 2 * seg)
                names = list(range(k * GS, (k + 2) * GS))
                u = lambda r, lo, hi: jnp.concatenate([u_p[p, r, :] for p in range(lo, hi)], axis=1)
                cols = lambda f: jnp.concatenate([f(n) for n in range(KP)], axis=1)
                part = {}

                def last_panel():
                    a = u(both, NP - 1, NP).astype(BF16)
                    r = pl.ds((NP - 1) * LANES // 2, LANES // 2)
                    for n in range(ND - 1):
                        part[n] = _dot(a, weight(wout_v, n, r))

                def last_columns():
                    silu(ND - 1, names, _dot(u(both, 0, NP).astype(BF16), weight(wout_v, ND - 1)))

                def product(p, add):
                    left, terms, _ = STRASSEN[p]
                    blocks = [[u(pl.ds((k + f) * seg, seg), c * YP, (c + 1) * YP) for c in range(2)] for f in range(2)]
                    if len(terms) > 1:
                        w = cols(lambda n: weight(wys_v, SUMS.index(p), n))
                    else:
                        r = pl.ds(terms[0][0] * YP * LANES // 2, YP * LANES // 2)
                        w = cols(lambda n: weight(wout_v, terms[0][1] * KP + n, r))
                    add(0, 0, _dot(_block_sum(blocks, left, _signed)[0][0].astype(BF16), w))

                def done(f, c, val):
                    for n in range(KP):
                        y = val[:, n * LANES:(n + 1) * LANES] + part[c * KP + n][f * seg:(f + 1) * seg]
                        silu(c * KP + n, names[f * GS:(f + 1) * GS], y)
                jobs = []
                _strassen(1, lambda p, add: jobs.append(functools.partial(product, p, add)), done, deferred=True)
                return [last_panel] + jobs[:4] + [last_columns] + jobs[4:]

            for op, g in schedule(k):
                dict(qkv=do_qkv, qk=do_qk, pv=do_pv, o=do_o, y=do_y)[op](g)

            if fast_o:
                for n in range(KP):
                    def done(f, c, val, n=n):
                        m = val.shape[0] // SUB
                        res.update(zip([(2 * n + c, g) for g in og[f * m:(f + 1) * m]], groups(val)))
                    _strassen(1, lambda p, add, n=n: add(0, 0, acc[p, n]() if opts.get('accv') else acc[p, n]), done)
            for n in range(ND - 1 if fast_o else 0, ND):
                res.update(zip([(n, g) for g in og], groups(acc[n]() if opts.get('accv') else acc[n])))
            mem = jnp.concatenate([res.pop((n, "m")) for n in range(ND)], axis=1)
            for g in range(0, U * GS, 2):
                if all((n, q) in res and (n, q) in gate for n in range(ND) for q in (g, g + 1)):
                    r = pl.ds(g * SUB, 2 * SUB)
                    val = rows([jnp.concatenate([res.pop((n, q)) * gate.pop((n, q)) for n in range(ND)], axis=1)
                                for q in (g, g + 1)])
                    out_p[r, :] = (x_p[r, :].astype(F32) + val).astype(BF16)
        assert not res and not gate and not gating
        cp_out(i).start()
        return mem

    if not opts.get('noa'):
      with jax.named_scope('A'):
        lax.fori_loop(0, n_seg // U, period, mem0_v[0].astype(F32))
    with jax.named_scope('waitout'):
        pltpu.make_async_copy(out_v, out_hbm.at[0], sem_out).wait()


def build(opts):
    @functools.partial(jax.jit, static_argnames=("A_seg_len",))
    def fn(A_x, A_mem0, A_Wq, A_Wk, A_Wv, A_Wo, A_seg_len, B_x, B_w_in, B_w_sp, B_b_sp, B_w_out):
        del B_x
        B, S, D = A_x.shape
        H, Dh = A_Wq.shape[1], A_Wq.shape[2]
        F = B_w_in.shape[1]
        Fh = F // 2
        NP = -(-Fh // LANES)
        TB = opts.get("tb", 512)
        n1 = S // TB
        n2 = S // (2 * LANES * opts.get("pairs", 2))
        ND = D // LANES
        NTT = S // LANES
        LV = opts.get("lv", 2)
        any_spec = pl.BlockSpec(memory_space=pl.ANY)
        vm = pl.BlockSpec(memory_space=pltpu.VMEM)
        dma = pltpu.SemaphoreType.DMA
        scratch = [
            pltpu.VMEM((S + 64, D), BF16),
            pltpu.VMEM((S, D), F32),
            pltpu.VMEM((F, D), BF16),
            pltpu.VMEM((NTT, S // 2, LANES), U32),
            pltpu.VMEM((ND, NP * LANES // 2, LANES), U32),
            pltpu.VMEM((NTT, Fh, LANES), F32),
            pltpu.VMEM((NTT, Fh + SUB, LANES), F32),
            pltpu.VMEM((NTT, SUB, LANES), F32),
            pltpu.VMEM((7 ** LV + 1 if not opts.get('aonly') else 2, NTT // 2 ** LV, Fh // 2 ** LV, LANES), F32),
            pltpu.VMEM((NP, S + opts.get('pu', 32), LANES), F32),
            pltpu.VMEM((6 * H // 16 + 1, D // 2 * SUB, Dh), U32),
            pltpu.VMEM((3, H, D // 2, Dh), U32),
            pltpu.VMEM((ND, H * Dh // 2, LANES), U32),
            pltpu.VMEM((S, D), BF16),
            pltpu.VMEM((H * 2 * opts.get('ks', 48) * opts.get('nkv', 2), Dh), F32),
            pltpu.SMEM((1,), jnp.int32),
            pltpu.VMEM((2, 8, (ND - 1) // 2, Fh // 4, LANES), U32),
            pltpu.VMEM((3, H // 2, len(SUMS), (ND - 1) // 2 * LANES // 2, Dh), U32),
            pltpu.VMEM((len(SUMS), (ND - 1) // 2, (NP - 1) // 2 * LANES // 2, LANES), U32),
            pltpu.VMEM(A_mem0.shape, BF16),
            pltpu.VMEM(B_b_sp.shape, BF16),
            pltpu.VMEM((opts.get("pad", 8), LANES), U32),
            dma((TB // opts.get('xc', 256),)), dma((n1 - 1,)), dma((2,)), dma(()), dma((n2,)), dma(()), dma(()),
        ]
        return pl.pallas_call(
            functools.partial(_kernel, seg=A_seg_len, S=S, H=H, opts=opts),
            out_shape=jax.ShapeDtypeStruct((B, S, D), A_x.dtype),
            in_specs=[any_spec] * 10,
            out_specs=any_spec,
            scratch_shapes=scratch,
            compiler_params=pltpu.CompilerParams(vmem_limit_bytes=opts.get("vmem", 126) * 2**20, flags=opts.get("flags", {"XLA_TPU_RESCHEDULE_DMA_DONES": True}),
                                                 disable_bounds_checks=opts.get("nobc", True),
                                                 disable_semaphore_checks=opts.get("nosc", False)),
        )(A_x, A_mem0, *[w.reshape(ND, LANES // 2, 2, H, Dh) for w in (A_Wq, A_Wk, A_Wv)], A_Wo.reshape(H * Dh, D), B_w_in.T, B_w_sp, B_b_sp, B_w_out)
    return fn


pallas_recurrent_scan__memory_aug_recurrent_mem_tr__mixer_gmlp__prompt_kernel = build({})
```

```python
import functools
import jax
import jax.numpy as jnp
import numpy as np
from jax import lax
import jax.experimental.pallas as pl
import jax.experimental.pallas.tpu as pltpu

F32 = jnp.float32
BF16 = jnp.bfloat16
U32 = jnp.uint32
NT = (((1,), (1,)), ((), ()))
LANES = 128
SUB = 8
EPS = 1e-5
LOG2E = 1.4426950408889634


STRASSEN = (
    (((0, 0, 1), (0, 1, 1)), ((1, 1, 1),), ((0, 0, -1), (0, 1, 1))),
    (((0, 0, 1),), ((0, 1, 1), (1, 1, -1)), ((0, 1, 1), (1, 1, 1))),
    (((1, 0, 1), (1, 1, 1)), ((0, 0, 1),), ((1, 0, 1), (1, 1, -1))),
    (((1, 1, 1),), ((1, 0, 1), (0, 0, -1)), ((0, 0, 1), (1, 0, 1))),
    (((0, 0, 1), (1, 1, 1)), ((0, 0, 1), (1, 1, 1)), ((0, 0, 1), (1, 1, 1))),
    (((0, 1, 1), (1, 1, -1)), ((1, 0, 1), (1, 1, 1)), ((0, 0, 1),)),
    (((1, 0, 1), (0, 0, -1)), ((0, 0, 1), (0, 1, 1)), ((1, 1, 1),)),
)


SPLIT_233 = (
    (((0, 0, 1),), ((0, 0, 1), (0, 2, -1), (2, 0, -1)), ((0, 0, 1),)),
    (((0, 1, 1), (1, 1, -1)), ((0, 2, 1), (1, 1, -1), (1, 2, -1)), ((1, 2, 1),)),
    (((0, 1, 1), (1, 0, -1), (1, 1, -1)), ((1, 0, 1), (0, 2, -1)), ((0, 0, 1), (0, 2, 1), (1, 2, 1))),
    (((0, 1, 1),), ((1, 2, 1), (2, 2, 1), (1, 0, -1)), ((0, 2, 1), (1, 2, 1))),
    (((1, 0, 1), (1, 1, 1), (0, 0, -1), (0, 1, -1)), ((0, 2, 1),), ((0, 0, -1), (0, 2, -1))),
    (((0, 1, 1), (0, 2, -1)), ((2, 2, 1),), ((0, 1, 1), (0, 2, -1))),
    (((1, 2, 1), (0, 1, -1)), ((1, 1, 1), (2, 2, -1)), ((0, 1, -1), (1, 2, -1))),
    (((1, 0, 1), (1, 1, 1)), ((1, 0, 1),), ((0, 0, 1), (0, 2, 1), (1, 0, 1), (1, 2, 1))),
    (((0, 0, 1), (0, 2, 1)), ((2, 0, 1),), ((0, 0, 1), (0, 1, 1), (1, 0, 1), (1, 1, 1))),
    (((1, 1, 1), (1, 2, -1)), ((1, 1, 1),), ((1, 1, 1), (1, 2, -1))),
    (((0, 0, 1), (0, 2, 1), (1, 2, -1)), ((2, 0, 1), (0, 1, -1)), ((0, 1, -1), (1, 0, -1), (1, 1, -1))),
    (((1, 2, 1),), ((1, 1, 1), (2, 1, 1), (2, 0, -1)), ((0, 1, 1), (1, 1, 1))),
    (((1, 2, 1), (0, 2, -1)), ((2, 1, 1), (2, 2, 1), (0, 1, -1)), ((0, 1, -1),)),
    (((1, 0, 1), (1, 2, 1), (0, 0, -1), (0, 2, -1)), ((0, 1, 1),), ((1, 0, 1), (1, 1, 1))),
    (((1, 0, 1),), ((0, 1, 1), (1, 0, 1), (0, 0, -1)), ((1, 0, -1),)),
)
SUMS_233 = tuple(p for p, (_, terms, _) in enumerate(SPLIT_233) if len(terms) > 1)


def _terms_sum(blocks, terms, f):
    total = blocks[terms[0][0]][terms[0][1]]
    for r, c, sign in terms[1:]:
        total = f(sign, total, blocks[r][c])
    return total


SUMS = tuple(p for p, (_, terms, _) in enumerate(STRASSEN) if len(terms) > 1)


def _block_sum(blocks, terms, f):
    h = len(blocks) // 2
    quad = lambda r, c: [row[c * h:(c + 1) * h] for row in blocks[r * h:(r + 1) * h]]
    first = quad(*terms[0][:2])
    if len(terms) == 1:
        return first
    return [[f(terms[1][2], x, y) for x, y in zip(rx, ry)] for rx, ry in zip(first, quad(*terms[1][:2]))]


def _signed(sign, x, y):
    return x + y if sign > 0 else x - y


def _halves(w):
    if isinstance(w, tuple):
        return w
    return pltpu.bitcast(w << 16, F32), pltpu.bitcast(w & jnp.uint32(0xFFFF0000), F32)


def _words(w):
    return pltpu.pack_elementwise(list(w), packed_dtype=BF16) if isinstance(w, tuple) else w


def _signed_halves(sign, x, y):
    return tuple(_signed(sign, p, q) for p, q in zip(_halves(x), _halves(y)))


def _strassen(h, product, emit, deferred=False, scheme=STRASSEN, start=None):
    acc = {}
    for p, (_, _, outs) in enumerate(scheme):
        later = {(r, c) for _, _, o in scheme[p + 1:] for r, c, _ in o}

        def add(r0, c0, val, outs=outs, later=later, p=p):
            if start and p == 0:
                acc.update({key: (1, v) for key, v in start().items()})
            for r, c, sign in outs:
                key = (r * h + r0, c * h + c0)
                if key not in acc:
                    acc[key] = (sign, val)
                elif acc[key][0] > 0:
                    acc[key] = (1, _signed(sign, acc[key][1], val))
                else:
                    acc[key] = (1, val - acc[key][1]) if sign > 0 else (-1, acc[key][1] + val)
                if (r, c) not in later:
                    emit(*key, acc.pop(key)[1])
        product(p, add)


def _lhs_sums(blocks):
    if len(blocks) == 1:
        return [blocks[0][0]]
    return [v for terms, _, _ in STRASSEN for v in _lhs_sums(_block_sum(blocks, terms, _signed))]


def _dot(a, b):
    return jnp.dot(a, b, preferred_element_type=F32)


def _dot_nt(a, b):
    return lax.dot_general(a, b, NT, preferred_element_type=F32)


def _gelu2(a):
    u = a * (0.7978845608028654 + (0.7978845608028654 * 0.044715) * (a * a))
    return a * (1.0 + jnp.tanh(u))


def _ds(start, size):
    if isinstance(start, int):
        return pl.ds(start, size)
    return pl.ds(pl.multiple_of(start, size), size)


def _kernel(x_hbm, mem0_hbm, wq_hbm, wk_hbm, wv_hbm, wo_hbm, win_hbm, wsp_hbm, bsp_hbm, wout_hbm,
            out_hbm,
            x_v, xn_v, win_v, wsp_v, wout_v, z1_v, z2_v, zm_v, zc_v, u_v,
            wraw_v, wqkv_v, wo_v, kv_v, row_s, wsum_v, wqs_v, wys_v, mem0_v, bsp_v, pad_v,
            sem_x0, sem_x, sem_win, sem_wsp, sem_w, sem_late, sem_out, *, seg, S, H, opts):
    D = x_v.shape[1]
    out_v = x_v.at[pl.ds(0, S)]
    M = mem0_hbm.shape[1]
    Dh = wq_hbm.shape[-1]
    F = win_hbm.shape[0]
    Fh = F // 2
    Fq = Fh // 2
    NP = u_v.shape[0]
    L = M + seg
    n_seg = S // seg
    ND = D // LANES
    TB = opts.get("tb", 512)
    n1 = S // TB
    NC = TB // LANES
    TT = 2 * LANES * opts.get("pairs", 2)
    n2 = S // TT
    DC = D // n2
    HP = H // 2
    NA = HP // SUB
    LV = opts.get("lv", 2)
    NB = 2 ** LV
    FB = Fh // NB

    XC = opts.get("xc", 256)

    def cp_x0(c):
        r = _ds(c * XC, XC)
        return pltpu.make_async_copy(x_hbm.at[0, r], x_v.at[r], sem_x0.at[c])

    def start_x(i):
        for c in range(0, TB, LANES):
            pltpu.make_async_copy(x_hbm.at[0, _ds(i * TB + c, LANES)], x_v.at[_ds(i * TB + c, LANES)],
                                  sem_x.at[i - 1]).start()

    def wait_x(i):
        blk = x_v.at[_ds(i * TB, TB)]
        pltpu.make_async_copy(blk, blk, sem_x.at[i - 1]).wait()

    def cp_win(i):
        r = pl.ds(i * Fh, Fh)
        return pltpu.make_async_copy(win_hbm.at[r], win_v.at[r], sem_win.at[i])

    NTT = S // LANES

    def cp_wsp(j):
        return pltpu.make_async_copy(wsp_hbm.bitcast(U32).at[:, _ds(j * LANES, LANES)], wsp_v.at[j], sem_wsp)

    KP = (ND - 1) // 2
    NT3 = H // 6 * 2
    YP = (NP - 1) // 2
    OB = H * Dh // 2 // n2
    DT = LANES // n2

    def cp_ws(i):
        r = pl.ds(i * DT // 2, DT // 2)
        dst = wraw_v.reshape(wraw_v.shape[0], ND, LANES // 2, SUB, Dh)
        return [pltpu.make_async_copy(w.bitcast(U32).at[:, r, par, pl.ds(a * SUB, SUB)],
                                      dst.at[2 * (t * NA + a) + par, :, r], sem_w.at[i])
                for t, w in enumerate((wq_hbm, wk_hbm, wv_hbm)) for a in range(NA) for par in range(2)]

    Fw = Fq // LANES * LANES
    Fr = Fq - Fw
    f_parts = [(0, 0, Fw), (Fq, Fw, Fw), (Fw, 2 * Fw, Fr), (Fq + Fw, 2 * Fw + Fr, Fr)]
    cp_wout = [pltpu.make_async_copy(wout_hbm.bitcast(U32).at[pl.ds(src // 2, n // 2), pl.ds(j * LANES, LANES)],
                                     wout_v.at[j, pl.ds(dst // 2, n // 2)], sem_wsp)
               for j in range(ND) for src, dst, n in f_parts]
    cp_late = [pltpu.make_async_copy(wo_hbm.bitcast(U32).at[:, pl.ds(j * LANES, LANES)], wo_v.at[j], sem_late)
                for j in range(ND)]
    cp_late.append(pltpu.make_async_copy(mem0_hbm, mem0_v, sem_late))
    cp_bias = pltpu.make_async_copy(bsp_hbm, bsp_v, sem_win.at[0])

    U = opts.get("unroll", 4)

    def cp_out(s):
        r = _ds(s * seg * U, seg * U)
        return pltpu.make_async_copy(out_v.at[r], out_hbm.at[0, r], sem_out)

    def first_copies(f, carry):
        for c in range(TB // XC // 2):
            cp_x0(f * (TB // XC // 2) + c).start()
        r = _ds(Fh + f * Fq, Fq)
        pltpu.make_async_copy(win_hbm.at[r], win_v.at[r], sem_win.at[1]).start()
        return carry
    lax.fori_loop(0, 2, first_copies, 0)

    wout_v[:, pl.ds(Fq, NP * LANES // 2 - Fq), :] = jnp.zeros((ND, NP * LANES // 2 - Fq, LANES), U32)
    KS, NKV = opts.get("ks", 48), opts.get("nkv", 2)
    for j in range(2 * H * NKV):
        kv_v[pl.ds(j * KS, SUB), :] = jnp.zeros((SUB, Dh), F32)

    def ln_x(start, rows):
        r = _ds(start, rows)
        x = x_v[r, :].astype(F32)
        c = x - jnp.mean(x, axis=-1, keepdims=True)
        v = jnp.mean(c * c, axis=-1, keepdims=True)
        xn_v[r, :] = c * lax.rsqrt(v + EPS)

    def win_sums(half):
        tile = lambda f, r, j: pltpu.bitcast(
            win_v[pl.ds((2 * half + f) * Fq + 2 * r, 2 * SUB), pl.ds(j * LANES, LANES)], U32)
        for r in range(0, Fq // 2, SUB):
            for j in range(KP):
                raw = [[tile(f, r, k * KP + j) for k in range(2)] for f in range(2)]
                split = [[_halves(w) for w in row] for row in raw]
                for p, (terms, _, _) in enumerate(STRASSEN):
                    val = _block_sum(split if len(terms) > 1 else raw, terms, _signed_halves)[0][0]
                    wsum_v[half, p, j, pl.ds(r, SUB)] = _words(val)
            for f in range(2):
                wsum_v[half, 7, f, pl.ds(r, SUB)] = tile(f, r, ND - 1)

    def hidden(half, i, emit, busy):
        xn = lambda c, lo, n: xn_v[_ds(i * TB + c * LANES, LANES), pl.ds(lo * LANES, n * LANES)]
        w_last = pltpu.bitcast(jnp.concatenate([wsum_v[half, 7, f] for f in range(2)], axis=0), BF16)
        blocks = [[jnp.concatenate([xn(c, k * KP, KP) for c in range(c1, NC, 2)], axis=0) for c1 in range(2)]
                  for k in range(2)]
        last = _dot_nt(w_last, jnp.concatenate([xn(c, ND - 1, 1) for c in range(NC)], axis=0).astype(BF16))
        busy(0, last)

        def product(p, add):
            lhs = [wsum_v[half, p, j] for j in range(KP)]
            d = _dot_nt(jnp.concatenate([pltpu.bitcast(w, BF16) for w in lhs], axis=1),
                        _block_sum(blocks, STRASSEN[p][1], _signed)[0][0].astype(BF16))
            add(0, 0, d)
            busy(p + 1, d)

        def done(f, c1, val):
            for n, c in enumerate(range(c1, NC, 2)):
                emit(f, c, val[:, n * LANES:(n + 1) * LANES] + last[f * Fq:(f + 1) * Fq, c * LANES:(c + 1) * LANES])
        _strassen(1, product, done)

    def first_block(c, carry):
        cp_x0(c).wait()
        if opts.get("x1pos", 1) >= 0:
            @pl.when(c == opts.get("x1pos", 1))
            def _():
                start_x(1)
        ln_x(c * XC, XC)
        return carry
    with jax.named_scope('start'):
        lax.fori_loop(0, TB // XC, first_block, 0)
    with jax.named_scope('waitwin'):
        cp_win(1).wait()
    if opts.get("x1pos", 1) < 0:
        start_x(1)
    win_sums(1)

    def p1(i, carry):
        RL = opts.get("rl", 8)
        MID, END = opts.get("mid", (2, 7))
        sums = {}

        def emit(f, c, pre):
            z = _gelu2(pre)
            z2_v[i * NC + c, pl.ds(f * Fq, Fq), :] = z
            part = jnp.sum(z.reshape(Fq // SUB, SUB, LANES), axis=0)
            if c in sums:
                mean = jnp.sum(sums[c] + part, axis=0, keepdims=True) * (1.0 / Fh)
                zm_v[i * NC + c] = jnp.broadcast_to(mean, (SUB, LANES))
            sums[c] = part

        def busy(n, d):
            if n == MID:
                pl.when(i + 1 < n1)(lambda: wait_x(i + 1))
                first = opts.get("wsp0", 4)
                for it in range(n1):
                    @pl.when(i == it)
                    def _(it=it):
                        if it == 0:
                            for b in range(2, n1):
                                start_x(b)
                            cp_win(0).start()
                            cp_bias.start()
                        cut = lambda k: first + k * (NTT - first) // (n1 - 1) if k >= 0 else 0
                        for j in range(cut(it - 1), cut(it)):
                            cp_wsp(j).start()
            if MID <= n < END:
                mine = range((n - MID) * (TB // RL) // (END - MID), (n + 1 - MID) * (TB // RL) // (END - MID))
                for m, piece in enumerate(mine):
                    r0 = (m * d.shape[0] // len(mine)) // 16 * 16
                    x_v[_ds(S + (i % 2) * 16, 16), pl.ds(0, LANES)] = d[r0:r0 + 16, :LANES].astype(BF16)
                    ln_x(jnp.minimum(i + 1, n1 - 1) * TB + piece * RL, RL)
        hidden(1, i, emit, busy)

        return carry
    if not opts.get('aonly'):
      with jax.named_scope('P1'):
        lax.fori_loop(0, n1, p1, 0)

    cp_win(0).wait()
    cp_bias.wait()
    win_sums(0)
    for cp in cp_wout + cp_ws(0):
        cp.start()

    U2 = opts.get("u2", 1)

    def p2(ii, carry):
      for i in [ii * U2 + b for b in range(U2)]:
        var, rstd = {}, {}
        rows = range(0, FB, SUB)
        work = []
        for g in range(NC // NB):
            work += [("var", g, r) for r in rows] + [("rstd", g, 0)] + [("norm", g, r) for r in rows]
        nvar = opts.get("nvar", 28)

        def emit(f, c, pre):
            z1_v[i * NC + c, pl.ds(f * Fq, Fq), :] = _gelu2(pre)

        def busy(n, d):
            share = opts.get("share", (1, 2, 3, 4, 5, 6, 7))
            rest = len(work) - nvar
            cut = lambda k: nvar + (share[k - 1] * rest // share[-1] if k else 0)
            mine = work[cut(n - 1):cut(n)] if n else work[:nvar]
            for m, (kind, g, r) in enumerate(mine):
                t0 = i * NC + g * NB
                if kind == "rstd":
                    for e in range(NB):
                        ss = jnp.broadcast_to(jnp.sum(var[g, e], axis=0, keepdims=True), (SUB, LANES))
                        rstd[g, e] = 0.5 * lax.rsqrt(ss * (1.0 / Fh) + 4.0 * EPS)
                    continue
                r0 = m * d.shape[0] // len(mine) // SUB * SUB
                z2_v[i % 3, pl.ds(Fh, SUB), :] = d[r0:r0 + SUB, :LANES]
                a = [[z2_v[t0 + e, pl.ds(f * FB + r, SUB), :] - zm_v[t0 + e] for e in range(NB)] for f in range(NB)]
                if kind == "var":
                    for e in range(NB):
                        sq = functools.reduce(lambda x, y: x + y, [a[f][e] * a[f][e] for f in range(NB)])
                        var[g, e] = var[g, e] + sq if (g, e) in var else sq
                else:
                    a = [[a[f][e] * rstd[g, e] for e in range(NB)] for f in range(NB)]
                    burst = opts.get("burst", 11)
                    for q, val in enumerate(_lhs_sums(a)):
                        if q and q % burst == 0:
                            r1 = (m * 7 ** LV + q) * d.shape[0] // 7 ** LV // len(mine) // SUB * SUB
                            zc_v[7 ** LV, i % 3, pl.ds(0, SUB), :] = d[r1:r1 + SUB, :LANES]
                        zc_v[q, i * (NC // NB) + g, pl.ds(r, SUB), :] = val
        hidden(0, i, emit, busy)

        @pl.when(i == opts.get("w1", n1 - 1))
        def _():
            for cp in cp_ws(1) + cp_late[:1]:
                cp.start()

      return carry
    if not opts.get('aonly'):
      with jax.named_scope('P2'):
        lax.fori_loop(0, n1 // U2, p2, 0)

    for cp in [cp_wsp(j) for j in range(NTT)] + cp_wout:
        cp.wait()

    RC = opts.get("rc", 16)

    def p3(i, carry):
        with jax.named_scope('wW'):
            for cp in cp_ws(i):
                cp.wait()

        RB = DT // 2
        here = lambda ref, *lead, scale=1: ref.at[(*lead, pl.ds(
            pl.multiple_of(i * RB * scale, RB * scale), ref.shape[len(lead)] - (n2 - 1) * RB * scale))]
        al = slice(None)
        raw_p, wqkv_p, wqs_p, wqt_p = here(wraw_v, al, scale=SUB), here(wqkv_v, al, al), here(wqs_v, al, al, al), here(z2_v, al)
        wout_p, wys_p = here(wout_v, al, scale=YP), here(wys_v, al, al, scale=YP)

        def raw(t, j, r):
            a, jj = divmod(j, SUB)
            return [raw_p[2 * (t * NA + a) + par, pl.ds(r * SUB + jj, SUB, stride=SUB), :] for par in range(2)]

        at = lambda n, e: n * LANES // 2 + e * SUB
        put = lambda n, e: pl.ds(at(n, e), SUB)

        def split_heads(t, j, e, panels):
            for n in panels:
                even, odd = raw(t, j, at(n, e))
                wqkv_p[t, 2 * j, put(n, e)] = pltpu.pack_elementwise([even, odd], packed_dtype=jnp.uint16)
                wqkv_p[t, 2 * j + 1, put(n, e)] = (even >> 16) | (odd & jnp.uint32(0xFFFF0000))

        def head_sums(t, n, e):
            if n < NT3:
                blocks = [[_halves(wqkv_p[t, 3 * n + c, put(r, e)]) for c in range(3)] for r in range(3)]
                sums = [SPLIT_233[p][1] for p in SUMS_233]
            else:
                blocks = [[_halves(wqkv_p[t, 3 * n + c, put(r, e)]) for c in range(2)] for r in range(2)]
                sums = [STRASSEN[p][1] for p in SUMS]
            for m, terms in enumerate(sums):
                wqs_p[t, n, m, put(0, e)] = _words(_terms_sum(blocks, terms, _signed_halves))

        def tail_sums(t, j, e):
            blocks = []
            for n in range(3, ND):
                even, odd = [_halves(w) for w in raw(t, j, at(n, e))]
                blocks.append([(even[c], odd[c]) for c in range(2)])
                for c in range(2):
                    wqkv_p[t, 2 * j + c, put(n, e)] = _words(blocks[-1][c])
            for n, p in enumerate(SUMS):
                val = _words(_terms_sum(blocks, STRASSEN[p][1], _signed_halves))
                wqt_p[j, put(t * len(SUMS) + n, e)] = pltpu.bitcast(val, F32)

        def out_sums(j, e):
            blocks = [[_halves(wout_p[c * KP + j, put(k * YP, e)]) for c in range(2)] for k in range(2)]
            for n, p in enumerate(SUMS):
                wys_p[n, j, put(0, e)] = _words(_terms_sum(blocks, STRASSEN[p][1], _signed_halves))

        rl = []
        for e in range(DT // (2 * SUB)):
            for t in range(3):
                for j in range(HP):
                    rl += [(0, functools.partial(split_heads, t, j, e, range(3))), (0, functools.partial(tail_sums, t, j, e))]
                    rl += [(1, functools.partial(head_sums, t, n, e)) for n in range(NT3 + 1)
                           if min(3 * n + 2, H - 1) // 2 == j]
        extra = [(0, functools.partial(out_sums, j, e)) for j in range(KP) for e in range(YP * LANES // 2 // n2 // SUB)]
        for n, piece in enumerate(extra):
            rl.insert((n + 1) * len(rl) // (len(extra) + 1), piece)

        n_grp = TT // (NB * LANES)
        KJ = S // LANES // NB
        n_job = n_grp * 7 ** LV * (KJ // 4)
        state = [0]
        posts = []

        def leaf(q, rhs, emit):
            acc = None
            for h in range(KJ // 4):
                js = range(4 * h, 4 * h + 4)
                d = _dot_nt(jnp.concatenate([zc_v[q, j] for j in js], axis=1),
                            jnp.concatenate([pltpu.bitcast(_words(rhs[j]()), BF16) for j in js], axis=1))
                acc = d if acc is None else acc + d
                n = state[0]
                state[0] += 1
                mine = rl[n * len(rl) // n_job:(n + 1) * len(rl) // n_job]
                early = len(posts)
                if h == KJ // 4 - 1:
                    emit(0, 0, acc)
                for m, piece in enumerate(mine):
                    r0 = (m * FB // len(mine)) // SUB * SUB
                    tick = d[r0:r0 + SUB]
                    if piece[0]:
                        if opts.get("t2", True):
                            wqkv_v[i % 3, H, pl.ds(0, SUB)] = pltpu.bitcast(tick, U32)
                    else:
                        wraw_v[6 * NA, _ds(i * SUB, SUB), :] = pltpu.bitcast(tick, U32)
                    piece[1]()
                    if early and m % opts.get("pp", 3) == 0:
                        u_v[i % NP, pl.ds(S, SUB), :] = tick
                        posts.pop(0)()
                        early -= 1

        def lazy_sum(sign, x, y):
            def one(a, b):
                memo = []

                def get():
                    if not memo:
                        memo.append(_signed_halves(sign, a(), b()))
                    return memo[0]
                return get
            return [one(a, b) for a, b in zip(x, y)]

        def products(q, rhs, emit):
            if len(rhs) == 1:
                return leaf(q, rhs[0][0], emit)
            _strassen(len(rhs) // 2,
                      lambda p, add: products(q * 7 + p, _block_sum(rhs, STRASSEN[p][1], lazy_sum), add), emit)

        for gi in range(n_grp):
            t0 = i * TT + gi * NB * LANES
            bias = 0.5 * bsp_v[_ds(t0, NB * LANES)].astype(F32).reshape(1, NB * LANES)
            g, todo = {}, []

            def w(e, c, j, t0=t0):
                return lambda: wsp_v[NB * j + e, _ds((t0 + c * LANES) // 2, LANES // 2), :]

            for c in range(NB):
                for f in range(2):
                    for j in range(Fw // LANES):
                        todo.append((f * (Fw // LANES) + j, c, [(f * Fq + j * LANES, f * Fq + (j + 1) * LANES)]))
                todo.append((NP - 1, c, [(Fw, Fq), (Fq + Fw, Fh)]))

            def post(p, c, spans, t0=t0, bias=bias, g=g):
                parts = []
                for lo, hi in spans:
                    for f in range(lo // FB, (hi - 1) // FB + 1):
                        a, b = max(lo, f * FB), min(hi, (f + 1) * FB)
                        z1 = z1_v[t0 // LANES + c, pl.ds(a, b - a), :]
                        parts.append(z1 * (g[f, c][a - f * FB:b - f * FB] + bias[:, c * LANES:(c + 1) * LANES]))
                n = sum(x.shape[0] for x in parts)
                if n < LANES:
                    parts.append(jnp.zeros((LANES - n, LANES), F32))
                u_v[p, _ds(t0 + c * LANES, LANES), :] = jnp.concatenate(parts, axis=0).T

            def finished(f, c, val, g=g, todo=todo, post=post):
                g[f, c] = val
                for item in list(todo):
                    need = {(ff, item[1]) for lo, hi in item[2] for ff in range(lo // FB, (hi - 1) // FB + 1)}
                    if need <= set(g):
                        todo.remove(item)
                        posts.append(functools.partial(post, *item))

            products(0, [[[w(e, c, j) for j in range(KJ)] for c in range(NB)] for e in range(NB)], finished)
        for p in posts:
            p()

        for it, cps in enumerate((cp_ws(2) + cp_late[1:2], cp_ws(3) + cp_late[2:3], cp_late[3:])):
            @pl.when(i == it)
            def _(cps=cps):
                for cp in cps:
                    cp.start()

        return carry
    if not opts.get('aonly') and not opts.get('bonly'):
      with jax.named_scope('P3'):
        lax.fori_loop(0, n2, p3, 0)

    for c in cp_late:
        c.wait()

    c2 = Dh ** (-0.5) * LOG2E
    NEG = -1e9 * LOG2E
    G = opts.get("G", 4)
    NG = H // G
    GS = seg // SUB
    row_s[0] = 2 * H * KS

    def recip(x):
        r = pl.reciprocal(x, approx=True)
        return r * (2.0 - x * r)

    def chain(f, xs):
        return functools.reduce(f, xs)

    plain = [(False, range(k * GS, (k + 1) * GS)) for k in range(U)]
    q_plan = [(True, range(0, 7)), (False, range(7, 10)), (False, range(10, 13)), (False, range(13, 16))]
    o_plan = [(False, range(0, 3)), (False, range(3, 6)), (False, range(6, 9)), (True, range(9, 16))]
    if not opts.get("sq", True): q_plan = plain
    if opts.get("p64"): q_plan = [(False, g) for _, g in q_plan]
    if not opts.get("so", False): o_plan = plain
    if opts.get("lagged"):
        if opts.get("so", False):
            o_plan = [(False, (1, 2, 3)), (False, (0, 5, 6)), (False, (4, 7, 9)), (True, (8, 10, 11, 12, 13, 14, 15))]
        else:
            o_plan = [(False, (1, 2, 3)), (False, (0, 5, 6, 7)), (False, (4, 9, 10, 11)), (False, (8, 12, 13, 14, 15))]

    ahead = [g for k, (_, gs) in enumerate(q_plan) for g in gs if g >= (k + 1) * GS]

    def schedule(k):
        ne, lag = opts.get("early", (3, 4)) if k < U - 1 else opts.get("early_last", (3, 5))
        if k == 0: ne, lag = opts.get("early_first", (ne, lag))
        order = opts.get("inner", "xqpo")
        seq = []
        for t in range(NG):
            for w in order:
                if w == "x": seq.append(("qkv", t))
                if w == "q" and t >= 1: seq.append(("qk", t - 1))
                if w == "p" and t >= 2: seq.append(("pv", t - 2))
                if w == "o" and 0 <= t - lag < ne: seq.append(("o", t - lag))
        tail = opts.get("tail", "o3 q7 o4 o5 p6 p7 y0 o6 y1 o7 y2 y3")
        if k == U - 1:
            tail = opts.get("tail_last", "y0 y1 y2 o3 q7 o4 p6 o5 y3 p7 o6 o7")
        if k == 0: tail = opts.get("tail_first", tail)
        names = dict(o="o", q="qk", p="pv", y="y")
        return seq + [(names[w[0]], int(w[1:])) for w in tail.split()]

    def groups(a):
        return [a[r:r + SUB] for r in range(0, a.shape[0], SUB)]

    def rows(parts):
        return jnp.concatenate(parts, axis=0)

    def lhs(a, kind):
        return a.astype(BF16) if a.shape[0] % (2 * SUB) == 0 and kind in opts.get("pack", "h") else a

    def period(i, mem):
        row = lax.broadcasted_iota(jnp.int32, (L - SUB, L), 0)
        col = lax.broadcasted_iota(jnp.int32, (L - SUB, L), 1)
        mask = (row < M) | (row + SUB >= col)
        sub = lax.broadcasted_iota(jnp.int32, (SUB, 1), 0)
        proj = {}
        att = {}
        gate, res, gating = {}, {}, []

        tokens = _ds(i * U * seg, U * seg)
        xn_p, x_p, u_p, out_p = xn_v.at[tokens], x_v.at[tokens], u_v.at[:, tokens], out_v.at[tokens]

        def xn(g):
            return xn_p[pl.ds(g * SUB, SUB), :]

        for k in range(U):
            fast_q, qg = q_plan[k]
            fast_o, og = o_plan[k]
            qg, og = ["m"] + list(qg), ["m"] + list(og)
            keys = ["m"] + list(range(k * GS, (k + 1) * GS))
            h = rows([mem] + [xn(g) for g in qg[1:]])
            sc, acc, us, jobs = {}, {}, [], []
            if fast_q:
                n = h.shape[0] // 2
                blocks = [[h[f * n:(f + 1) * n, c * LANES:(c + 1) * LANES] for c in range(ND)] for f in range(2)]
                h_head = [_terms_sum(blocks, terms, _signed).astype(BF16) for terms, _, _ in SPLIT_233]
                h_rest = [_terms_sum(blocks, terms, _signed).astype(BF16) for terms, _, _ in STRASSEN]
                h_tail = [_terms_sum([row[3:] for row in blocks], terms, _signed).astype(BF16) for terms, _, _ in STRASSEN]
            else:
                h = lhs(h, 'h')

            def keep(t, hd, names, vals):
                for g, val in zip(names, vals):
                    if g in keys or not opts.get("carry", True):
                        proj[t, hd, g] = val
                    else:
                        z1_v[8 + ahead.index(g), pl.ds((t * H + hd) * SUB, SUB), :] = val
                for g in keys:
                    if g not in names and opts.get("carry", True):
                        proj[t, hd, g] = z1_v[8 + ahead.index(g), pl.ds((t * H + hd) * SUB, SUB), :]

            def weight(ref, *idx):
                return pltpu.bitcast(ref[idx], BF16)

            def fast_jobs():
                panel = lambda n: pl.ds(n * LANES // 2, LANES // 2)
                part = {}
                todo = {(t, hd): 2 if hd < 3 * NT3 else 3 for t in range(3) for hd in range(H)}
                jobs = []

                def add_part(f, t, hd, val):
                    part[f, t, hd] = val
                    if f == 1 and (0, t, hd) in part or f == 0 and (1, t, hd) in part:
                        todo[t, hd] -= 1
                        if not todo[t, hd]:
                            keep(t, hd, qg, groups(part.pop((0, t, hd))) + groups(part.pop((1, t, hd))))
                            if not any(todo[u, hd] for u in range(3)):
                                first_rows(hd)

                def scheme(table, left, t, hd0, panel0, summed):
                    sums = [p for p, (_, terms, _) in enumerate(table) if len(terms) > 1]
                    width = 1 + max(c for _, _, outs in table for _, c, _ in outs)
                    steps = []

                    def product(p, add):
                        terms = table[p][1]
                        w = summed(sums.index(p)) if len(terms) > 1 else weight(
                            wqkv_v, t, hd0 + terms[0][1], panel(panel0 + terms[0][0]))
                        add(0, 0, _dot(left[p], w))

                    def start():
                        return {(f, c): part.pop((f, t, hd0 + c)) for f in range(2) for c in range(width)
                                if (f, t, hd0 + c) in part}
                    _strassen(1, lambda p, add: steps.append(functools.partial(product, p, add)),
                              lambda f, c, val: add_part(f, t, hd0 + c, val), scheme=table, start=start)
                    jobs.extend(steps)

                first = lambda t, n: scheme(SPLIT_233, h_head, t, 3 * n, 0, lambda m: weight(wqs_v, t, n, m))
                last = lambda t, j: scheme(STRASSEN, h_tail, t, 2 * j, 3,
                                           lambda m: weight(z2_v, j, panel(t * len(SUMS) + m)))
                for n in range(0, NT3, 2):
                    j = n // 2 * 3
                    seq = ((first, n), (last, j), (last, j + 1), (last, j + 2), (first, n + 1))
                    if opts.get("tmaj"):
                        for part_ in (seq[:3], seq[3:]):
                            for t in range(3):
                                for f, a in part_:
                                    f(t, a)
                        continue
                    for f, a in seq:
                        for t in range(3):
                            f(t, a)
                for t in range(3):

                    def middle(hd, t=t):
                        d = _dot(h[:, 2 * LANES:3 * LANES], weight(wqkv_v, t, hd, panel(2)))
                        for f in range(2):
                            add_part(f, t, hd, d[f * d.shape[0] // 2:(f + 1) * d.shape[0] // 2])
                    jobs.extend(functools.partial(middle, hd) for hd in range(3 * NT3, H))
                    scheme(STRASSEN, h_rest, t, 3 * NT3, 0, lambda m, t=t: weight(wqs_v, t, NT3, m))
                    last(t, H // 2 - 1)
                return jobs

            def first_rows(hd):
                kbase = (k % NKV * H + hd) * 2 * KS + SUB
                vbase = kbase + KS
                nk = len(keys) if opts.get("allkv", 1) else 2
                kv_v[pl.ds(kbase, nk * SUB), :] = rows([proj[1, hd, g] for g in keys[:nk]])
                kv_v[pl.ds(vbase, nk * SUB), :] = rows([proj[2, hd, g] for g in keys[:nk]])
                if opts.get("stq", 1):
                    slab, n0 = divmod(k % 2 * H + hd, Fh // L)
                    z1_v[slab, pl.ds(n0 * L, L), :] = rows([proj[0, hd, g] for g in keys])
                    for n, g in enumerate(keys):
                        proj[0, hd, g] = z1_v[slab, pl.ds(n0 * L + n * SUB, SUB), :]
                if opts.get("allkv", 1):
                    for n, g in enumerate(keys):
                        proj[1, hd, g] = kv_v[pl.ds(kbase + n * SUB, SUB), :]
                        proj[2, hd, g] = kv_v[pl.ds(vbase + n * SUB, SUB), :]
                qs = proj[0, hd, keys[1]] * c2
                ts = range(M, -SUB, -1)
                z = [jnp.sum(qs * kv_v[pl.ds(kbase + t, SUB), :], axis=-1, keepdims=True) for t in ts]
                z = [zt if t >= 0 else jnp.where(sub >= -t, zt, NEG) for zt, t in zip(z, ts)]
                mx = chain(jnp.maximum, z)
                e = [jnp.exp2(zt - mx) for zt in z]
                den = chain(jnp.add, e)
                num = chain(jnp.add, [et * kv_v[pl.ds(vbase + t, SUB), :] for et, t in zip(e, ts)])
                att[hd, keys[1]] = num * recip(den)

            def do_qkv(g):
                if fast_q:
                    if not g:
                        jobs.extend(fast_jobs())
                    while any((hd, keys[1]) not in att for hd in range(g * G, (g + 1) * G)):
                        jobs.pop(0)()
                    return
                for j in range(g * G // 2, (g + 1) * G // 2):
                    for t in opts.get("qkvo", (0, 1, 2)):
                        for hd in (2 * j, 2 * j + 1):
                            keep(t, hd, qg, groups(_dot(h, weight(wqkv_v, t, hd))))
                    for hd in (2 * j, 2 * j + 1):
                        first_rows(hd)

            def do_qk(g):
                for hd in range(g * G, (g + 1) * G):
                    q = rows([proj[0, hd, r] for r in keys[:1] + keys[2:]])
                    sc[hd] = _dot_nt(lhs(q, 'q'), rows([proj[1, hd, r] for r in keys]).astype(BF16))

            def do_pv(g):
                for hd in range(g * G, (g + 1) * G):
                    z = jnp.where(mask, sc[hd] * c2, NEG)
                    e = jnp.exp2(z - jnp.max(z, axis=-1, keepdims=True))
                    p = e * recip(jnp.sum(e, axis=-1, keepdims=True))
                    o = _dot(lhs(p, 'p'), rows([proj[2, hd, r] for r in keys]).astype(BF16))
                    att.update(zip([(hd, r) for r in keys[:1] + keys[2:]], groups(o)))

            def accumulate(key, d):
                if opts.get("accv", 1):
                    slot = key if isinstance(key, int) else ND + key[0] * KP + key[1]
                    r = pl.ds(slot * 64 if slot < ND else ND * 64 + (slot - ND) * 32, d.shape[0])
                    z1_v[14 + k % 2, r, :] = z1_v[14 + k % 2, r, :] + d if key in acc else d
                    acc[key] = functools.partial(lambda r: z1_v[14 + k % 2, r, :], r)
                else:
                    acc[key] = acc[key] + d if key in acc else d

            def do_o(g):
                for j in range(g * G // 2, (g + 1) * G // 2):
                    o = [rows([att[2 * j + c, r] for r in og]) for c in range(2)]
                    head = lambda c: pl.ds((2 * j + c) * (Dh // 2), Dh // 2)
                    if not fast_o:
                        for c in range(2):
                            a = lhs(o[c], 'o')
                            for n in range(ND):
                                accumulate(n, _dot(a, weight(wo_v, n, head(c))))
                        continue
                    half = o[0].shape[0] // 2
                    blocks = [[o[c][f * half:(f + 1) * half] for c in range(2)] for f in range(2)]
                    for c in range(2):
                        accumulate(ND - 1, _dot(lhs(o[c], 'o'), weight(wo_v, ND - 1, head(c))))
                    for p, (left, terms, _) in enumerate(STRASSEN):
                        a = lhs(_block_sum(blocks, left, _signed)[0][0], 'o')
                        for n in range(KP):
                            if len(terms) > 1:
                                w = pltpu.bitcast(z2_v[j, pl.ds((n * len(SUMS) + SUMS.index(p)) * (Dh // 2), Dh // 2), :], BF16)
                            else:
                                w = weight(wo_v, 2 * n + terms[0][1], head(terms[0][0]))
                            accumulate((p, n), _dot(a, w))

            def silu(n, names, y):
                hy = 0.5 * y
                gate.update(zip([(n, r) for r in names], groups(hy + hy * jnp.tanh(hy))))

            def do_y(j):
                if not opts.get("sy", True):
                    if not us:
                        us.append(jnp.concatenate([u_p[p, pl.ds(k * seg, seg), :] for p in range(NP)], axis=1).astype(BF16))
                    silu(j, keys[1:], _dot(us[0], weight(wout_v, j)))
                    return
                if k % 2 == 0 and j == 0:
                    gating[:] = gate_jobs(k)
                for _ in range(2 if k % 2 == 0 and j == opts.get("dbl", 3) else 1):
                    if gating:
                        gating.pop(0)()

            def gate_jobs(k):
                both = pl.ds(k * seg, 2 * seg)
                names = list(range(k * GS, (k + 2) * GS))
                u = lambda r, lo, hi: jnp.concatenate([u_p[p, r, :] for p in range(lo, hi)], axis=1)
                cols = lambda f: jnp.concatenate([f(n) for n in range(KP)], axis=1)
                part = {}

                def last_panel():
                    a = u(both, NP - 1, NP).astype(BF16)
                    r = pl.ds((NP - 1) * LANES // 2, LANES // 2)
                    for n in range(ND - 1):
                        part[n] = _dot(a, weight(wout_v, n, r))

                def last_columns():
                    silu(ND - 1, names, _dot(u(both, 0, NP).astype(BF16), weight(wout_v, ND - 1)))

                def product(p, add):
                    left, terms, _ = STRASSEN[p]
                    blocks = [[u(pl.ds((k + f) * seg, seg), c * YP, (c + 1) * YP) for c in range(2)] for f in range(2)]
                    if len(terms) > 1:
                        w = cols(lambda n: weight(wys_v, SUMS.index(p), n))
                    else:
                        r = pl.ds(terms[0][0] * YP * LANES // 2, YP * LANES // 2)
                        w = cols(lambda n: weight(wout_v, terms[0][1] * KP + n, r))
                    add(0, 0, _dot(_block_sum(blocks, left, _signed)[0][0].astype(BF16), w))

                def done(f, c, val):
                    for n in range(KP):
                        y = val[:, n * LANES:(n + 1) * LANES] + part[c * KP + n][f * seg:(f + 1) * seg]
                        silu(c * KP + n, names[f * GS:(f + 1) * GS], y)
                jobs = []
                _strassen(1, lambda p, add: jobs.append(functools.partial(product, p, add)), done, deferred=True)
                return [last_panel] + jobs[:4] + [last_columns] + jobs[4:]

            for op, g in schedule(k):
                dict(qkv=do_qkv, qk=do_qk, pv=do_pv, o=do_o, y=do_y)[op](g)

            if fast_o:
                for n in range(KP):
                    def done(f, c, val, n=n):
                        m = val.shape[0] // SUB
                        res.update(zip([(2 * n + c, g) for g in og[f * m:(f + 1) * m]], groups(val)))
                    _strassen(1, lambda p, add, n=n: add(0, 0, acc[p, n]() if opts.get('accv', 1) else acc[p, n]), done)
            for n in range(ND - 1 if fast_o else 0, ND):
                res.update(zip([(n, g) for g in og], groups(acc[n]() if opts.get('accv', 1) else acc[n])))
            mem = jnp.concatenate([res.pop((n, "m")) for n in range(ND)], axis=1)
            for g in range(0, U * GS, 2):
                if all((n, q) in res and (n, q) in gate for n in range(ND) for q in (g, g + 1)):
                    r = pl.ds(g * SUB, 2 * SUB)
                    val = rows([jnp.concatenate([res.pop((n, q)) * gate.pop((n, q)) for n in range(ND)], axis=1)
                                for q in (g, g + 1)])
                    out_p[r, :] = (x_p[r, :].astype(F32) + val).astype(BF16)
        assert not res and not gate and not gating
        cp_out(i).start()
        return mem

    if not opts.get('noa'):
      with jax.named_scope('A'):
        lax.fori_loop(0, n_seg // U, period, mem0_v[0].astype(F32))
    with jax.named_scope('waitout'):
        pltpu.make_async_copy(out_v, out_hbm.at[0], sem_out).wait()


def build(opts):
    @functools.partial(jax.jit, static_argnames=("A_seg_len",))
    def fn(A_x, A_mem0, A_Wq, A_Wk, A_Wv, A_Wo, A_seg_len, B_x, B_w_in, B_w_sp, B_b_sp, B_w_out):
        del B_x
        B, S, D = A_x.shape
        H, Dh = A_Wq.shape[1], A_Wq.shape[2]
        F = B_w_in.shape[1]
        Fh = F // 2
        NP = -(-Fh // LANES)
        TB = opts.get("tb", 512)
        n1 = S // TB
        n2 = S // (2 * LANES * opts.get("pairs", 2))
        ND = D // LANES
        NTT = S // LANES
        LV = opts.get("lv", 2)
        any_spec = pl.BlockSpec(memory_space=pl.ANY)
        vm = pl.BlockSpec(memory_space=pltpu.VMEM)
        dma = pltpu.SemaphoreType.DMA
        scratch = [
            pltpu.VMEM((S + 64, D), BF16),
            pltpu.VMEM((S, D), F32),
            pltpu.VMEM((F, D), BF16),
            pltpu.VMEM((NTT, S // 2, LANES), U32),
            pltpu.VMEM((ND, NP * LANES // 2, LANES), U32),
            pltpu.VMEM((NTT, Fh, LANES), F32),
            pltpu.VMEM((NTT, max(Fh + SUB, 3 * len(SUMS) * LANES // 2), LANES), F32),
            pltpu.VMEM((NTT, SUB, LANES), F32),
            pltpu.VMEM((7 ** LV + 1 if not opts.get('aonly') else 2, NTT // 2 ** LV, Fh // 2 ** LV, LANES), F32),
            pltpu.VMEM((NP, S + opts.get('pu', 32), LANES), F32),
            pltpu.VMEM((6 * H // 16 + 1, D // 2 * SUB, Dh), U32),
            pltpu.VMEM((3, H + 1, D // 2, Dh), U32),
            pltpu.VMEM((ND, H * Dh // 2, LANES), U32),
            pltpu.VMEM((H * 2 * opts.get('ks', 48) * opts.get('nkv', 2), Dh), F32),
            pltpu.SMEM((1,), jnp.int32),
            pltpu.VMEM((2, 8, (ND - 1) // 2, Fh // 4, LANES), U32),
            pltpu.VMEM((3, H // 3 + 1, len(SUMS_233), LANES // 2, Dh), U32),
            pltpu.VMEM((len(SUMS), (ND - 1) // 2, (NP - 1) // 2 * LANES // 2, LANES), U32),
            pltpu.VMEM(A_mem0.shape, BF16),
            pltpu.VMEM(B_b_sp.shape, BF16),
            pltpu.VMEM((opts.get("pad", 8), LANES), U32),
            dma((TB // opts.get('xc', 256),)), dma((n1 - 1,)), dma((2,)), dma(()), dma((n2,)), dma(()), dma(()),
        ]
        return pl.pallas_call(
            functools.partial(_kernel, seg=A_seg_len, S=S, H=H, opts=opts),
            out_shape=jax.ShapeDtypeStruct((B, S, D), A_x.dtype),
            in_specs=[any_spec] * 10,
            out_specs=any_spec,
            scratch_shapes=scratch,
            compiler_params=pltpu.CompilerParams(vmem_limit_bytes=opts.get("vmem", 126) * 2**20, flags=opts.get("flags", {"XLA_TPU_RESCHEDULE_DMA_DONES": True}),
                                                 disable_bounds_checks=opts.get("nobc", True),
                                                 disable_semaphore_checks=opts.get("nosc", False)),
        )(A_x, A_mem0, *[w.reshape(ND, LANES // 2, 2, H, Dh) for w in (A_Wq, A_Wk, A_Wv)], A_Wo.reshape(H * Dh, D), B_w_in.T, B_w_sp, B_b_sp, B_w_out)
    return fn


pallas_recurrent_scan__memory_aug_recurrent_mem_tr__mixer_gmlp__prompt_kernel = build({})
```

```python
import functools

import jax
import jax.numpy as jnp
from jax import lax
import jax.experimental.pallas as pl
import jax.experimental.pallas.tpu as pltpu

F32 = jnp.float32
BF16 = jnp.bfloat16
U32 = jnp.uint32
LANES = 128
SUB = 8
WORDS = LANES // 2
EPS = 1e-5
LOG2E = 1.4426950408889634
GELU_A = 0.7978845608028654
GELU_B = GELU_A * 0.044715

TOKENS = 512
PERIOD = 4
GROUP = 4

STRASSEN = (
    (((0, 0, 1), (0, 1, 1)), ((1, 1, 1),), ((0, 0, -1), (0, 1, 1))),
    (((0, 0, 1),), ((0, 1, 1), (1, 1, -1)), ((0, 1, 1), (1, 1, 1))),
    (((1, 0, 1), (1, 1, 1)), ((0, 0, 1),), ((1, 0, 1), (1, 1, -1))),
    (((1, 1, 1),), ((1, 0, 1), (0, 0, -1)), ((0, 0, 1), (1, 0, 1))),
    (((0, 0, 1), (1, 1, 1)), ((0, 0, 1), (1, 1, 1)), ((0, 0, 1), (1, 1, 1))),
    (((0, 1, 1), (1, 1, -1)), ((1, 0, 1), (1, 1, 1)), ((0, 0, 1),)),
    (((1, 0, 1), (0, 0, -1)), ((0, 0, 1), (0, 1, 1)), ((1, 1, 1),)),
)
SPLIT_233 = (
    (((0, 0, 1),), ((0, 0, 1), (0, 2, -1), (2, 0, -1)), ((0, 0, 1),)),
    (((0, 1, 1), (1, 1, -1)), ((0, 2, 1), (1, 1, -1), (1, 2, -1)), ((1, 2, 1),)),
    (((0, 1, 1), (1, 0, -1), (1, 1, -1)), ((1, 0, 1), (0, 2, -1)), ((0, 0, 1), (0, 2, 1), (1, 2, 1))),
    (((0, 1, 1),), ((1, 2, 1), (2, 2, 1), (1, 0, -1)), ((0, 2, 1), (1, 2, 1))),
    (((1, 0, 1), (1, 1, 1), (0, 0, -1), (0, 1, -1)), ((0, 2, 1),), ((0, 0, -1), (0, 2, -1))),
    (((0, 1, 1), (0, 2, -1)), ((2, 2, 1),), ((0, 1, 1), (0, 2, -1))),
    (((1, 2, 1), (0, 1, -1)), ((1, 1, 1), (2, 2, -1)), ((0, 1, -1), (1, 2, -1))),
    (((1, 0, 1), (1, 1, 1)), ((1, 0, 1),), ((0, 0, 1), (0, 2, 1), (1, 0, 1), (1, 2, 1))),
    (((0, 0, 1), (0, 2, 1)), ((2, 0, 1),), ((0, 0, 1), (0, 1, 1), (1, 0, 1), (1, 1, 1))),
    (((1, 1, 1), (1, 2, -1)), ((1, 1, 1),), ((1, 1, 1), (1, 2, -1))),
    (((0, 0, 1), (0, 2, 1), (1, 2, -1)), ((2, 0, 1), (0, 1, -1)), ((0, 1, -1), (1, 0, -1), (1, 1, -1))),
    (((1, 2, 1),), ((1, 1, 1), (2, 1, 1), (2, 0, -1)), ((0, 1, 1), (1, 1, 1))),
    (((1, 2, 1), (0, 2, -1)), ((2, 1, 1), (2, 2, 1), (0, 1, -1)), ((0, 1, -1),)),
    (((1, 0, 1), (1, 2, 1), (0, 0, -1), (0, 2, -1)), ((0, 1, 1),), ((1, 0, 1), (1, 1, 1))),
    (((1, 0, 1),), ((0, 1, 1), (1, 0, 1), (0, 0, -1)), ((1, 0, -1),)),
)


def _summed(table):
    return tuple(p for p, (_, terms, _) in enumerate(table) if len(terms) > 1)


SUMS = _summed(STRASSEN)
SUMS_233 = _summed(SPLIT_233)

PROJECTED = (range(0, 7), range(7, 10), range(10, 13), range(13, 16))
ORDER = ((3, 4, "o3 q7 o4 o5 p6 p7 y0 o6 y1 o7 y2 y3"),) * 3 + ((3, 5, "y0 y1 q7 o3 o4 p6 y2 y3 o5 p7 o6 o7"),)


def _dot(a, b):
    return jnp.dot(a, b, preferred_element_type=F32)


def _dot_nt(a, b):
    return lax.dot_general(a, b, (((1,), (1,)), ((), ())), preferred_element_type=F32)


def _ds(start, size):
    return pl.ds(start if isinstance(start, int) else pl.multiple_of(start, size), size)


def _gelu2(a):
    return a * (1.0 + jnp.tanh(a * (GELU_A + GELU_B * (a * a))))


def _recip(x):
    r = pl.reciprocal(x, approx=True)
    return r * (2.0 - x * r)


def _signed(sign, x, y):
    return x + y if sign > 0 else x - y


def _halves(w):
    if isinstance(w, tuple):
        return w
    return pltpu.bitcast(w << 16, F32), pltpu.bitcast(w & jnp.uint32(0xFFFF0000), F32)


def _words(w):
    return pltpu.pack_elementwise(list(w), packed_dtype=BF16) if isinstance(w, tuple) else w


def _signed_halves(sign, x, y):
    return tuple(_signed(sign, p, q) for p, q in zip(_halves(x), _halves(y)))


def _terms_sum(blocks, terms, f):
    total = blocks[terms[0][0]][terms[0][1]]
    for r, c, sign in terms[1:]:
        total = f(sign, total, blocks[r][c])
    return total


def _quadrant_sum(grid, terms, f):
    h = len(grid) // 2
    quadrants = [[[row[c * h:(c + 1) * h] for row in grid[r * h:(r + 1) * h]] for c in range(2)] for r in range(2)]
    each = lambda sign, x, y: [[f(sign, a, b) for a, b in zip(rx, ry)] for rx, ry in zip(x, y)]
    return _terms_sum(quadrants, terms, each)


def _left_sums(grid):
    if len(grid) == 1:
        return [grid[0][0]]
    return [v for terms, _, _ in STRASSEN for v in _left_sums(_quadrant_sum(grid, terms, _signed))]


def _block_products(table, product, emit, h=1, start=None):
    acc = {}
    for p, (_, _, outs) in enumerate(table):
        later = [(r, c) for _, _, o in table[p + 1:] for r, c, _ in o]

        def add(r0, c0, val, outs=outs, later=later, p=p):
            if start and p == 0:
                acc.update({key: (1, v) for key, v in start().items()})
            for r, c, sign in outs:
                key = (r * h + r0, c * h + c0)
                if key not in acc:
                    acc[key] = (sign, val)
                elif acc[key][0] > 0:
                    acc[key] = (1, _signed(sign, acc[key][1], val))
                else:
                    acc[key] = (1, val - acc[key][1]) if sign > 0 else (-1, acc[key][1] + val)
                if (r, c) not in later:
                    sign, total = acc.pop(key)
                    assert sign > 0
                    emit(*key, total)
        product(p, add)


def _groups(a):
    return [a[r:r + SUB] for r in range(0, a.shape[0], SUB)]


def _rows(parts):
    return jnp.concatenate(parts, axis=0)


def _kernel(x_hbm, mem0_hbm, wq_hbm, wk_hbm, wv_hbm, wo_hbm, win_hbm, wsp_hbm, bsp_hbm, wout_hbm,
            out_hbm,
            x_v, xn_v, win_v, wsp_v, wout_v, z1_v, z2_v, zm_v, zc_v, u_v,
            wraw_v, wqkv_v, wo_v, kv_v, wsum_v, wqs_v, wys_v, mem0_v, bsp_v,
            sem_x0, sem_x, sem_win, sem_wsp, sem_w, sem_late, sem_out, *, seg):
    S, D = xn_v.shape
    M = mem0_hbm.shape[1]
    H, Dh = wq_hbm.shape[-2:]
    Fh = win_hbm.shape[0] // 2
    Fq = Fh // 2
    ND = D // LANES
    NP = u_v.shape[0]
    KP = (ND - 1) // 2
    YP = (NP - 1) // 2
    NB = TOKENS // LANES
    FB = Fh // NB
    n_blk = S // TOKENS
    NA = H // 2 // SUB
    out_v = x_v.at[pl.ds(0, S)]


    XC = TOKENS // 2

    def cp_x0(c):
        r = _ds(c * XC, XC)
        return pltpu.make_async_copy(x_hbm.at[0, r], x_v.at[r], sem_x0.at[c])

    def start_x(i):
        for c in range(0, TOKENS, LANES):
            r = _ds(i * TOKENS + c, LANES)
            pltpu.make_async_copy(x_hbm.at[0, r], x_v.at[r], sem_x.at[i - 1]).start()

    def wait_x(i):
        block = x_v.at[_ds(i * TOKENS, TOKENS)]
        pltpu.make_async_copy(block, block, sem_x.at[i - 1]).wait()

    def cp_win(half):
        r = pl.ds(half * Fh, Fh)
        return pltpu.make_async_copy(win_hbm.at[r], win_v.at[r], sem_win.at[half])

    def cp_wsp(j):
        return pltpu.make_async_copy(wsp_hbm.bitcast(U32).at[:, _ds(j * LANES, LANES)], wsp_v.at[j], sem_wsp)

    RB = WORDS // n_blk

    def cp_w(i):
        r = pl.ds(i * RB, RB)
        dst = wraw_v.reshape(wraw_v.shape[0], ND, WORDS, SUB, Dh)
        return [pltpu.make_async_copy(w.bitcast(U32).at[:, r, odd, pl.ds(a * SUB, SUB)],
                                      dst.at[2 * (t * NA + a) + odd, :, r], sem_w.at[i])
                for t, w in enumerate((wq_hbm, wk_hbm, wv_hbm)) for a in range(NA) for odd in range(2)]

    Fw = Fq // LANES * LANES
    parts = [(0, 0, Fw), (Fq, Fw, Fw), (Fw, 2 * Fw, Fq - Fw), (Fq + Fw, Fw + Fq, Fq - Fw)]
    cp_wout = [pltpu.make_async_copy(wout_hbm.bitcast(U32).at[pl.ds(src // 2, n // 2), pl.ds(j * LANES, LANES)],
                                     wout_v.at[j, pl.ds(dst // 2, n // 2)], sem_wsp)
               for j in range(ND) for src, dst, n in parts]
    cp_late = [pltpu.make_async_copy(wo_hbm.bitcast(U32).at[:, pl.ds(j * LANES, LANES)], wo_v.at[j], sem_late)
               for j in range(ND)]
    cp_late.append(pltpu.make_async_copy(mem0_hbm, mem0_v, sem_late))
    cp_bias = pltpu.make_async_copy(bsp_hbm, bsp_v, sem_win.at[0])

    def first_copies(f, carry):
        cp_x0(f).start()
        r = _ds(Fh + f * Fq, Fq)
        pltpu.make_async_copy(win_hbm.at[r], win_v.at[r], sem_win.at[1]).start()
        return carry
    lax.fori_loop(0, 2, first_copies, 0)

    wout_v[:, pl.ds(Fq, NP * WORDS - Fq), :] = jnp.zeros((ND, NP * WORDS - Fq, LANES), U32)
    KS = SUB + M + seg
    for j in range(kv_v.shape[0] // KS):
        kv_v[pl.ds(j * KS, SUB), :] = jnp.zeros((SUB, Dh), F32)

    def ln_x(start, n):
        r = _ds(start, n)
        x = x_v[r, :].astype(F32)
        c = x - jnp.mean(x, axis=-1, keepdims=True)
        v = jnp.mean(c * c, axis=-1, keepdims=True)
        xn_v[r, :] = c * lax.rsqrt(v + EPS)

    def win_sums(half):
        tile = lambda f, r, j: pltpu.bitcast(
            win_v[pl.ds((2 * half + f) * Fq + 2 * r, 2 * SUB), pl.ds(j * LANES, LANES)], U32)
        for r in range(0, Fq // 2, SUB):
            for j in range(KP):
                raw = [[tile(f, r, k * KP + j) for k in range(2)] for f in range(2)]
                split = [[_halves(w) for w in row] for row in raw]
                for p, (terms, _, _) in enumerate(STRASSEN):
                    val = _terms_sum(split if len(terms) > 1 else raw, terms, _signed_halves)
                    wsum_v[half, p, j, pl.ds(r, SUB)] = _words(val)
            for f in range(2):
                wsum_v[half, len(STRASSEN), f, pl.ds(r, SUB)] = tile(f, r, ND - 1)

    def hidden(half, i, emit, busy):
        xn = lambda c, lo, n: xn_v[_ds(i * TOKENS + c * LANES, LANES), pl.ds(lo * LANES, n * LANES)]
        w_last = pltpu.bitcast(_rows([wsum_v[half, len(STRASSEN), f] for f in range(2)]), BF16)
        blocks = [[_rows([xn(c, k * KP, KP) for c in range(c1, NB, 2)]) for c1 in range(2)] for k in range(2)]
        last = _dot_nt(w_last, _rows([xn(c, ND - 1, 1) for c in range(NB)]).astype(BF16))
        busy(0, last)

        def product(p, add):
            left = [wsum_v[half, p, j] for j in range(KP)]
            d = _dot_nt(jnp.concatenate([pltpu.bitcast(w, BF16) for w in left], axis=1),
                        _terms_sum(blocks, STRASSEN[p][1], _signed).astype(BF16))
            add(0, 0, d)
            busy(p + 1, d)

        def done(f, c1, val):
            for n, c in enumerate(range(c1, NB, 2)):
                emit(f, c, val[:, n * LANES:(n + 1) * LANES] + last[f * Fq:(f + 1) * Fq, c * LANES:(c + 1) * LANES])
        _block_products(STRASSEN, product, done)

    def first_block(c, carry):
        cp_x0(c).wait()
        pl.when(c == 1)(lambda: start_x(1))
        ln_x(c * XC, XC)
        return carry
    lax.fori_loop(0, 2, first_block, 0)
    cp_win(1).wait()
    win_sums(1)

    def second_half(i, carry):
        sums = {}

        def emit(f, c, pre):
            z = _gelu2(pre)
            z2_v[i * NB + c, pl.ds(f * Fq, Fq), :] = z
            part = jnp.sum(z.reshape(Fq // SUB, SUB, LANES), axis=0)
            if c in sums:
                mean = jnp.sum(sums[c] + part, axis=0, keepdims=True) * (1.0 / Fh)
                zm_v[i * NB + c] = jnp.broadcast_to(mean, (SUB, LANES))
            sums[c] = part

        def busy(n, d):
            first, end = 2, 7
            if n == first:
                pl.when(i + 1 < n_blk)(lambda: wait_x(i + 1))
                for it in range(n_blk):
                    @pl.when(i == it)
                    def _(it=it):
                        if it == 0:
                            for b in range(2, n_blk):
                                start_x(b)
                            cp_win(0).start()
                            cp_bias.start()
                        for j in range(it * NB, (it + 1) * NB):
                            cp_wsp(j).start()
            if first <= n < end:
                cut = lambda k: (k - first) * (TOKENS // SUB) // (end - first)
                mine = range(cut(n), cut(n + 1))
                for m, piece in enumerate(mine):
                    r0 = (m * d.shape[0] // len(mine)) // (2 * SUB) * (2 * SUB)
                    x_v[_ds(S + (i % 2) * 2 * SUB, 2 * SUB), pl.ds(0, LANES)] = d[r0:r0 + 2 * SUB, :LANES].astype(BF16)
                    ln_x(jnp.minimum(i + 1, n_blk - 1) * TOKENS + piece * SUB, SUB)
        hidden(1, i, emit, busy)
        return carry
    lax.fori_loop(0, n_blk, second_half, 0)

    cp_win(0).wait()
    cp_bias.wait()
    win_sums(0)
    for cp in cp_wout + cp_w(0):
        cp.start()

    def first_half(i, carry):
        var, rstd = {}, {}
        measure = [("var", r) for r in range(0, FB, SUB)] + [("rstd", 0)]
        apply = [("norm", r) for r in range(0, FB, SUB)]
        n_sums = zc_v.shape[0] - 1

        def emit(f, c, pre):
            z1_v[i * NB + c, pl.ds(f * Fq, Fq), :] = _gelu2(pre)

        def busy(n, d):
            cut = lambda k: k * len(apply) // len(STRASSEN)
            mine = apply[cut(n - 1):cut(n)] if n else measure
            for m, (kind, r) in enumerate(mine):
                if kind == "rstd":
                    for e in range(NB):
                        ss = jnp.broadcast_to(jnp.sum(var[e], axis=0, keepdims=True), (SUB, LANES))
                        rstd[e] = 0.5 * lax.rsqrt(ss * (1.0 / Fh) + 4.0 * EPS)
                    continue
                r0 = m * d.shape[0] // len(mine) // SUB * SUB
                z2_v[i % 3, pl.ds(Fh, SUB), :] = d[r0:r0 + SUB, :LANES]
                a = [[z2_v[i * NB + e, pl.ds(f * FB + r, SUB), :] - zm_v[i * NB + e] for e in range(NB)]
                     for f in range(NB)]
                if kind == "var":
                    for e in range(NB):
                        sq = functools.reduce(jnp.add, [a[f][e] * a[f][e] for f in range(NB)])
                        var[e] = var[e] + sq if e in var else sq
                else:
                    a = [[a[f][e] * rstd[e] for e in range(NB)] for f in range(NB)]
                    for q, val in enumerate(_left_sums(a)):
                        if q and q % 11 == 0:
                            r1 = (m * n_sums + q) * d.shape[0] // n_sums // len(mine) // SUB * SUB
                            zc_v[n_sums, i % 3, pl.ds(0, SUB), :] = d[r1:r1 + SUB, :LANES]
                        zc_v[q, i, pl.ds(r, SUB), :] = val
        hidden(0, i, emit, busy)

        @pl.when(i == n_blk - 1)
        def _():
            for cp in cp_w(1) + cp_late[:1]:
                cp.start()
        return carry
    lax.fori_loop(0, n_blk, first_half, 0)

    for cp in [cp_wsp(j) for j in range(S // LANES)] + cp_wout:
        cp.wait()

    def gating(i, carry):
        for cp in cp_w(i):
            cp.wait()

        here = lambda ref, lead, scale=1: ref.at[(slice(None),) * lead + (pl.ds(
            pl.multiple_of(i * RB * scale, RB * scale), ref.shape[lead] - (n_blk - 1) * RB * scale),)]
        raw_p, wqkv_p, wqs_p, wqt_p = here(wraw_v, 1, SUB), here(wqkv_v, 2), here(wqs_v, 3), here(z2_v, 1)
        wout_p, wys_p = here(wout_v, 1, YP), here(wys_v, 2, YP)
        put = lambda n, e: pl.ds(n * WORDS + e * SUB, SUB)

        def raw(t, j, n, e):
            a, jj = divmod(j, SUB)
            r = pl.ds((n * WORDS + e * SUB) * SUB + jj, SUB, stride=SUB)
            return [raw_p[2 * (t * NA + a) + odd, r, :] for odd in range(2)]

        def split_heads(t, j, e):
            for n in range(3):
                even, odd = raw(t, j, n, e)
                wqkv_p[t, 2 * j, put(n, e)] = pltpu.pack_elementwise([even, odd], packed_dtype=jnp.uint16)
                wqkv_p[t, 2 * j + 1, put(n, e)] = (even >> 16) | (odd & jnp.uint32(0xFFFF0000))

        def head_sums(t, n, e):
            table, width = (SPLIT_233, 3) if 3 * n + 3 <= H else (STRASSEN, 2)
            blocks = [[_halves(wqkv_p[t, 3 * n + c, put(r, e)]) for c in range(width)] for r in range(width)]
            for m, p in enumerate(_summed(table)):
                wqs_p[t, n, m, put(0, e)] = _words(_terms_sum(blocks, table[p][1], _signed_halves))

        def tail_sums(t, j, e):
            blocks = []
            for n in range(3, ND):
                even, odd = [_halves(w) for w in raw(t, j, n, e)]
                blocks.append([(even[c], odd[c]) for c in range(2)])
                for c in range(2):
                    wqkv_p[t, 2 * j + c, put(n, e)] = _words(blocks[-1][c])
            for n, p in enumerate(SUMS):
                val = _words(_terms_sum(blocks, STRASSEN[p][1], _signed_halves))
                wqt_p[j, put(t * len(SUMS) + n, e)] = pltpu.bitcast(val, F32)

        def out_sums(j, e):
            blocks = [[_halves(wout_p[c * KP + j, put(k * YP, e)]) for c in range(2)] for k in range(2)]
            for n, p in enumerate(SUMS):
                wys_p[n, j, put(0, e)] = _words(_terms_sum(blocks, STRASSEN[p][1], _signed_halves))

        pieces = []
        for e in range(RB // SUB):
            for t in range(3):
                for j in range(H // 2):
                    pieces += [(False, functools.partial(split_heads, t, j, e)),
                               (False, functools.partial(tail_sums, t, j, e))]
                    pieces += [(True, functools.partial(head_sums, t, n, e)) for n in range(wqs_v.shape[1])
                               if min(3 * n + 2, H - 1) // 2 == j]
        extra = [(False, functools.partial(out_sums, j, e)) for j in range(KP) for e in range(YP * RB // SUB)]
        for n, piece in enumerate(extra):
            pieces.insert((n + 1) * len(pieces) // (len(extra) + 1), piece)

        n_products = zc_v.shape[0] - 1
        issued, posts = [0], []

        def leaf(q, right, emit):
            d = _dot_nt(jnp.concatenate([zc_v[q, j] for j in range(n_blk)], axis=1),
                        jnp.concatenate([pltpu.bitcast(_words(w()), BF16) for w in right], axis=1))
            n = issued[0]
            issued[0] += 1
            mine = pieces[n * len(pieces) // n_products:(n + 1) * len(pieces) // n_products]
            waiting = len(posts)
            emit(0, 0, d)
            for m, (reads_tiles, work) in enumerate(mine):
                r0 = (m * FB // len(mine)) // SUB * SUB
                tick = d[r0:r0 + SUB]
                if reads_tiles:
                    wqkv_v[i % 3, H, pl.ds(0, SUB)] = pltpu.bitcast(tick, U32)
                else:
                    wraw_v[6 * NA, _ds(i * SUB, SUB), :] = pltpu.bitcast(tick, U32)
                work()
                if waiting and m % 3 == 0:
                    u_v[i % NP, pl.ds(S, SUB), :] = tick
                    posts.pop(0)()
                    waiting -= 1

        def lazy_sum(sign, x, y):
            def one(a, b):
                memo = []

                def get():
                    if not memo:
                        memo.append(_signed_halves(sign, a(), b()))
                    return memo[0]
                return get
            return [one(a, b) for a, b in zip(x, y)]

        def products(q, grid, emit):
            if len(grid) == 1:
                return leaf(q, grid[0][0], emit)
            _block_products(
                STRASSEN, lambda p, add: products(q * 7 + p, _quadrant_sum(grid, STRASSEN[p][1], lazy_sum), add),
                emit, h=len(grid) // 2)

        t0 = i * TOKENS
        bias = 0.5 * bsp_v[_ds(t0, TOKENS)].astype(F32).reshape(1, TOKENS)
        g, todo = {}, []

        def w_tile(e, c, j):
            return lambda: wsp_v[NB * j + e, _ds((t0 + c * LANES) // 2, WORDS), :]

        for c in range(NB):
            for f in range(2):
                for j in range(Fw // LANES):
                    todo.append((f * (Fw // LANES) + j, c, [(f * Fq + j * LANES, f * Fq + (j + 1) * LANES)]))
            todo.append((NP - 1, c, [(Fw, Fq), (Fq + Fw, Fh)]))

        def post(p, c, spans):
            ut = []
            for lo, hi in spans:
                for f in range(lo // FB, (hi - 1) // FB + 1):
                    a, b = max(lo, f * FB), min(hi, (f + 1) * FB)
                    z1 = z1_v[t0 // LANES + c, pl.ds(a, b - a), :]
                    ut.append(z1 * (g[f, c][a - f * FB:b - f * FB] + bias[:, c * LANES:(c + 1) * LANES]))
            n = sum(part.shape[0] for part in ut)
            if n < LANES:
                ut.append(jnp.zeros((LANES - n, LANES), F32))
            u_v[p, _ds(t0 + c * LANES, LANES), :] = _rows(ut).T

        def finished(f, c, val):
            g[f, c] = val
            for item in list(todo):
                if all((ff, item[1]) in g for lo, hi in item[2] for ff in range(lo // FB, (hi - 1) // FB + 1)):
                    todo.remove(item)
                    posts.append(functools.partial(post, *item))

        products(0, [[[w_tile(e, c, j) for j in range(n_blk)] for c in range(NB)] for e in range(NB)], finished)
        for work in posts:
            work()

        for it, copies in enumerate((cp_w(2) + cp_late[1:2], cp_w(3) + cp_late[2:3], cp_late[3:])):
            @pl.when(i == it)
            def _(copies=copies):
                for cp in copies:
                    cp.start()
        return carry
    lax.fori_loop(0, n_blk, gating, 0)

    for cp in cp_late:
        cp.wait()

    L = M + seg
    GS = seg // SUB
    NG = H // GROUP
    scale = Dh ** -0.5 * LOG2E
    masked = -1e9 * LOG2E
    threes = H // 6 * 6
    ahead = [g for k, gs in enumerate(PROJECTED) for g in gs if g >= (k + 1) * GS]
    panel = lambda n: pl.ds(n * WORDS, WORDS)
    weight = lambda ref, *idx: pltpu.bitcast(ref[idx], BF16)

    def period(i, mem):
        row = lax.broadcasted_iota(jnp.int32, (L - SUB, L), 0)
        col = lax.broadcasted_iota(jnp.int32, (L - SUB, L), 1)
        mask = (row < M) | (row + SUB >= col)
        sub = lax.broadcasted_iota(jnp.int32, (SUB, 1), 0)
        proj = {}
        att = {}
        gate, res, gate_todo = {}, {}, []
        tokens = _ds(i * PERIOD * seg, PERIOD * seg)
        xn_p, x_p, u_p, out_p = xn_v.at[tokens], x_v.at[tokens], u_v.at[:, tokens], out_v.at[tokens]

        for k in range(PERIOD):
            names = ["m"] + list(PROJECTED[k])
            keys = ["m"] + list(range(k * GS, (k + 1) * GS))
            queries = keys[:1] + keys[2:]
            h = _rows([mem] + [xn_p[pl.ds(g * SUB, SUB), :] for g in names[1:]])
            scores, acc, jobs = {}, {}, []
            if k == 0:
                n = h.shape[0] // 2
                blocks = [[h[f * n:(f + 1) * n, c * LANES:(c + 1) * LANES] for c in range(ND)] for f in range(2)]
                h_head = [_terms_sum(blocks, terms, _signed).astype(BF16) for terms, _, _ in SPLIT_233]
                h_rest = [_terms_sum(blocks, terms, _signed).astype(BF16) for terms, _, _ in STRASSEN]
                h_tail = [_terms_sum([r[3:] for r in blocks], terms, _signed).astype(BF16) for terms, _, _ in STRASSEN]
            else:
                h = h.astype(BF16)

            def keep(t, hd, vals):
                slot = lambda g: (8 + ahead.index(g), pl.ds((t * H + hd) * SUB, SUB), slice(None))
                for g, val in zip(names, vals):
                    if g in keys:
                        proj[t, hd, g] = val
                    else:
                        z1_v[slot(g)] = val
                for g in keys:
                    if g not in names:
                        proj[t, hd, g] = z1_v[slot(g)]

            def first_rows(hd):
                kbase = (k % 2 * H + hd) * 2 * KS + SUB
                vbase = kbase + KS
                kv_v[pl.ds(kbase, L), :] = _rows([proj[1, hd, g] for g in keys])
                kv_v[pl.ds(vbase, L), :] = _rows([proj[2, hd, g] for g in keys])
                slab, n0 = divmod(k % 2 * H + hd, Fh // L)
                z1_v[slab, pl.ds(n0 * L, L), :] = _rows([proj[0, hd, g] for g in keys])
                for n, g in enumerate(keys):
                    proj[0, hd, g] = z1_v[slab, pl.ds(n0 * L + n * SUB, SUB), :]
                for n, g in enumerate(keys):
                    proj[1, hd, g] = kv_v[pl.ds(kbase + n * SUB, SUB), :]
                    proj[2, hd, g] = kv_v[pl.ds(vbase + n * SUB, SUB), :]
                qs = proj[0, hd, keys[1]] * scale
                ts = range(M, -SUB, -1)
                z = [jnp.sum(qs * kv_v[pl.ds(kbase + t, SUB), :], axis=-1, keepdims=True) for t in ts]
                z = [zt if t >= 0 else jnp.where(sub >= -t, zt, masked) for zt, t in zip(z, ts)]
                top = functools.reduce(jnp.maximum, z)
                e = [jnp.exp2(zt - top) for zt in z]
                den = functools.reduce(jnp.add, e)
                num = functools.reduce(jnp.add, [et * kv_v[pl.ds(vbase + t, SUB), :] for et, t in zip(e, ts)])
                att[hd, keys[1]] = num * _recip(den)

            def split_projection():
                part = {}
                left = {(t, hd): 2 if hd < threes else 3 for t in range(3) for hd in range(H)}
                todo = []

                def add_part(f, t, hd, val):
                    part[f, t, hd] = val
                    if (1 - f, t, hd) in part:
                        left[t, hd] -= 1
                        if not left[t, hd]:
                            keep(t, hd, _groups(part.pop((0, t, hd))) + _groups(part.pop((1, t, hd))))
                            if not any(left[u, hd] for u in range(3)):
                                first_rows(hd)

                def scheme(table, sums, t, hd0, panel0, stored):
                    width = 1 + max(c for _, _, outs in table for _, c, _ in outs)

                    def product(p, add):
                        terms = table[p][1]
                        w = stored(_summed(table).index(p)) if len(terms) > 1 else weight(
                            wqkv_v, t, hd0 + terms[0][1], panel(panel0 + terms[0][0]))
                        add(0, 0, _dot(sums[p], w))

                    def start():
                        return {(f, c): part.pop((f, t, hd0 + c)) for f in range(2) for c in range(width)
                                if (f, t, hd0 + c) in part}
                    _block_products(table, lambda p, add: todo.append(functools.partial(product, p, add)),
                                    lambda f, c, val: add_part(f, t, hd0 + c, val), start=start)

                first = lambda t, n: scheme(SPLIT_233, h_head, t, 3 * n, 0, lambda m: weight(wqs_v, t, n, m))
                last = lambda t, j: scheme(STRASSEN, h_tail, t, 2 * j, 3,
                                           lambda m: weight(z2_v, j, panel(t * len(SUMS) + m)))
                for n in range(0, threes // 3, 2):
                    j = n // 2 * 3
                    for f, a in ((first, n), (last, j), (last, j + 1), (last, j + 2), (first, n + 1)):
                        for t in range(3):
                            f(t, a)
                for t in range(3):

                    def middle(hd, t=t):
                        d = _dot(h[:, 2 * LANES:3 * LANES], weight(wqkv_v, t, hd, panel(2)))
                        for f in range(2):
                            add_part(f, t, hd, d[f * d.shape[0] // 2:(f + 1) * d.shape[0] // 2])
                    todo.extend(functools.partial(middle, hd) for hd in range(threes, H))
                    scheme(STRASSEN, h_rest, t, threes, 0, lambda m, t=t: weight(wqs_v, t, threes // 3, m))
                    last(t, H // 2 - 1)
                return todo

            def project(g):
                if k == 0:
                    if g == 0:
                        jobs.extend(split_projection())
                    while any((hd, keys[1]) not in att for hd in range(g * GROUP, (g + 1) * GROUP)):
                        jobs.pop(0)()
                    return
                for j in range(g * GROUP // 2, (g + 1) * GROUP // 2):
                    for t in (1, 2, 0):
                        for hd in (2 * j, 2 * j + 1):
                            keep(t, hd, _groups(_dot(h, weight(wqkv_v, t, hd))))
                    for hd in (2 * j, 2 * j + 1):
                        first_rows(hd)

            def score(g):
                for hd in range(g * GROUP, (g + 1) * GROUP):
                    q = _rows([proj[0, hd, r] for r in queries])
                    scores[hd] = _dot_nt(q, _rows([proj[1, hd, r] for r in keys]).astype(BF16))

            def attend(g):
                for hd in range(g * GROUP, (g + 1) * GROUP):
                    z = jnp.where(mask, scores[hd] * scale, masked)
                    e = jnp.exp2(z - jnp.max(z, axis=-1, keepdims=True))
                    p = e * _recip(jnp.sum(e, axis=-1, keepdims=True))
                    o = _dot(p, _rows([proj[2, hd, r] for r in keys]).astype(BF16))
                    att.update(zip([(hd, r) for r in queries], _groups(o)))

            total = lambda n: (14 + k % 2, pl.ds(n * WORDS, L), slice(None))

            def mix(g):
                for j in range(g * GROUP // 2, (g + 1) * GROUP // 2):
                    o = [_rows([att[2 * j + c, r] for r in keys]) for c in range(2)]
                    for c in range(2):
                        for n in range(ND):
                            d = _dot(o[c], weight(wo_v, n, pl.ds((2 * j + c) * (Dh // 2), Dh // 2)))
                            z1_v[total(n)] = z1_v[total(n)] + d if n in acc else d
                            acc[n] = True

            def silu(n, which, y):
                hy = 0.5 * y
                gate.update(zip([(n, r) for r in which], _groups(hy + hy * jnp.tanh(hy))))

            def gate_jobs(k):
                both = pl.ds(k * seg, 2 * seg)
                which = list(range(k * GS, (k + 2) * GS))
                u = lambda r, lo, hi: jnp.concatenate([u_p[p, r, :] for p in range(lo, hi)], axis=1)
                cols = lambda f: jnp.concatenate([f(n) for n in range(KP)], axis=1)
                part, todo = {}, []

                def last_panel():
                    a = u(both, NP - 1, NP).astype(BF16)
                    for n in range(ND - 1):
                        part[n] = _dot(a, weight(wout_v, n, panel(NP - 1)))

                def last_columns():
                    silu(ND - 1, which, _dot(u(both, 0, NP).astype(BF16), weight(wout_v, ND - 1)))

                def product(p, add):
                    left, terms, _ = STRASSEN[p]
                    grid = [[u(pl.ds((k + f) * seg, seg), c * YP, (c + 1) * YP) for c in range(2)] for f in range(2)]
                    if len(terms) > 1:
                        w = cols(lambda n: weight(wys_v, SUMS.index(p), n))
                    else:
                        r = pl.ds(terms[0][0] * YP * WORDS, YP * WORDS)
                        w = cols(lambda n: weight(wout_v, terms[0][1] * KP + n, r))
                    add(0, 0, _dot(_terms_sum(grid, left, _signed).astype(BF16), w))

                def done(f, c, val):
                    for n in range(KP):
                        y = val[:, n * LANES:(n + 1) * LANES] + part[c * KP + n][f * seg:(f + 1) * seg]
                        silu(c * KP + n, which[f * GS:(f + 1) * GS], y)
                _block_products(STRASSEN, lambda p, add: todo.append(functools.partial(product, p, add)), done)
                return [last_panel] + todo[:4] + [last_columns] + todo[4:]

            def gate_piece(j):
                if k % 2 == 0 and j == 0:
                    gate_todo.extend(gate_jobs(k))
                for _ in range(2 if k % 2 == 0 and j == 3 else 1):
                    gate_todo.pop(0)()

            early, delay, rest = ORDER[k]
            for g in range(NG):
                project(g)
                if g >= 1:
                    score(g - 1)
                if g >= 2:
                    attend(g - 2)
                if 0 <= g - delay < early:
                    mix(g - delay)
            for word in rest.split():
                dict(q=score, p=attend, o=mix, y=gate_piece)[word[0]](int(word[1:]))

            for n in range(ND):
                res.update(zip([(n, g) for g in keys], _groups(z1_v[total(n)])))
            mem = jnp.concatenate([res.pop((n, "m")) for n in range(ND)], axis=1)
            for g in range(0, PERIOD * GS, 2):
                if all((n, q) in res and (n, q) in gate for n in range(ND) for q in (g, g + 1)):
                    r = pl.ds(g * SUB, 2 * SUB)
                    val = _rows([jnp.concatenate([res.pop((n, q)) * gate.pop((n, q)) for n in range(ND)], axis=1)
                                 for q in (g, g + 1)])
                    out_p[r, :] = (x_p[r, :].astype(F32) + val).astype(BF16)
        assert not res and not gate and not gate_todo
        pltpu.make_async_copy(out_v.at[tokens], out_hbm.at[0, tokens], sem_out).start()
        return mem

    lax.fori_loop(0, S // (PERIOD * seg), period, mem0_v[0].astype(F32))
    pltpu.make_async_copy(out_v, out_hbm.at[0], sem_out).wait()


@functools.partial(jax.jit, static_argnames=("A_seg_len",))
def pallas_recurrent_scan__memory_aug_recurrent_mem_tr__mixer_gmlp__prompt_kernel(
    A_x: jax.Array,
    A_mem0: jax.Array,
    A_Wq: jax.Array,
    A_Wk: jax.Array,
    A_Wv: jax.Array,
    A_Wo: jax.Array,
    A_seg_len: int,
    B_x: jax.Array,
    B_w_in: jax.Array,
    B_w_sp: jax.Array,
    B_b_sp: jax.Array,
    B_w_out: jax.Array,
):
    del B_x
    B, S, D = A_x.shape
    M = A_mem0.shape[1]
    H, Dh = A_Wq.shape[1:]
    F = B_w_in.shape[1]
    Fh = F // 2
    ND, NP, NT = D // LANES, pl.cdiv(Fh, LANES), S // LANES
    n_blk = S // TOKENS
    assert (B, S, D, M, H, Dh, F, A_seg_len) == (1, 2048, 640, 8, 32, 128, 1728, 32)

    vmem, dma = pltpu.VMEM, pltpu.SemaphoreType.DMA
    scratch = [
        vmem((S + 64, D), BF16),
        vmem((S, D), F32),
        vmem((F, D), BF16),
        vmem((NT, S // 2, LANES), U32),
        vmem((ND, NP * WORDS, LANES), U32),
        vmem((NT, Fh, LANES), F32),
        vmem((NT, 3 * len(SUMS) * WORDS, LANES), F32),
        vmem((NT, SUB, LANES), F32),
        vmem((7 * 7 + 1, n_blk, Fh // 4, LANES), F32),
        vmem((NP, S + 32, LANES), F32),
        vmem((6 * H // 16 + 1, D // 2 * SUB, Dh), U32),
        vmem((3, H + 1, D // 2, Dh), U32),
        vmem((ND, H * Dh // 2, LANES), U32),
        vmem((2 * H * 2 * (SUB + M + A_seg_len), Dh), F32),
        vmem((2, 8, (ND - 1) // 2, Fh // 4, LANES), U32),
        vmem((3, H // 3 + 1, len(SUMS_233), WORDS, Dh), U32),
        vmem((len(SUMS), (ND - 1) // 2, (NP - 1) // 2 * WORDS, LANES), U32),
        vmem(A_mem0.shape, BF16),
        vmem(B_b_sp.shape, BF16),
        dma((2,)), dma((n_blk - 1,)), dma((2,)), dma(()), dma((n_blk,)), dma(()), dma(()),
    ]
    hbm = pl.BlockSpec(memory_space=pl.ANY)
    return pl.pallas_call(
        functools.partial(_kernel, seg=A_seg_len),
        out_shape=jax.ShapeDtypeStruct((B, S, D), A_x.dtype),
        in_specs=[hbm] * 10,
        out_specs=hbm,
        scratch_shapes=scratch,
        compiler_params=pltpu.CompilerParams(
            vmem_limit_bytes=126 * 2**20, flags={"XLA_TPU_RESCHEDULE_DMA_DONES": True}),
    )(A_x, A_mem0, *[w.reshape(ND, WORDS, 2, H, Dh) for w in (A_Wq, A_Wk, A_Wv)],
      A_Wo.reshape(H * Dh, D), B_w_in.T, B_w_sp, B_b_sp, B_w_out)
```
